```python
import os as _os
_os.environ.setdefault('JAX_PLATFORMS', 'cpu')
import jax
import jax.numpy as jnp

def _softmax(x, axis=-1):
    return jax.nn.softmax(x, axis=axis)

def _gelu(x):
    return jax.nn.gelu(x, approximate=True)

def _silu(x):
    return jax.nn.silu(x)

def _sigmoid(x):
    return jax.nn.sigmoid(x)

def _layernorm(x, axis=-1, eps=1e-05):
    m = jnp.mean(x, axis=axis, keepdims=True)
    v = jnp.var(x, axis=axis, keepdims=True)
    return (x - m) / jnp.sqrt(v + eps)

def _scatter_add(tgt, idx, src, axis=0):
    return tgt.at[idx].add(src)

def _segment_sum(src, seg, n):
    return jax.ops.segment_sum(src, seg, n)

class _Rng:

    def __init__(self, key):
        self._k = key

    def _next(self):
        self._k, sub = jax.random.split(self._k)
        return sub

    def normal(self, shape):
        return jax.random.normal(self._next(), shape, dtype=jnp.bfloat16)

    def randint(self, lo, hi, shape):
        return jax.random.randint(self._next(), shape, lo, hi, dtype=jnp.int32)

    def uniform(self, shape, lo=0.0, hi=1.0):
        return jax.random.uniform(self._next(), shape, jnp.bfloat16, lo, hi)

    def permutation(self, n):
        return jax.random.permutation(self._next(), n)
kernel_name = 'standalone__window_attn_twins__vision'

def setup_inputs():
    _rng = _Rng(jax.random.key(int.from_bytes(__import__("os").urandom(4), "little")))
    _w = lambda a: (lambda t: t.astype(jnp.bfloat16) if jnp.issubdtype(t.dtype, jnp.floating) else t)(jnp.asarray(a))
    H = W = 384 // 8 * 8
    C = 96
    return {'x': _w((lambda *s: _rng.normal(s) * 0.4)(1, H, W, C)), 'wq': _w((lambda *s: _rng.normal(s) * 0.4)(C, C)), 'wkv': _w((lambda *s: _rng.normal(s) * 0.4)(C, 2 * C)), 'wo': _w((lambda *s: _rng.normal(s) * 0.05)(C, C))}

def reference(x, wq, wkv, wo):
    B, H, W, C = x.shape
    win = 8
    nh, nw = (H // win, W // win)
    xs = x.reshape(B, nh, win, nw, win, C).mean(axis=(2, 4)).reshape(B, nh * nw, C)
    q = x.reshape(B, H * W, C) @ wq
    kv = xs @ wkv
    k, v = (kv[..., :C].copy(), kv[..., C:].copy())
    scale = C ** (-0.5)
    p = _softmax(jnp.einsum('bqc,bkc->bqk', q, k) * scale, axis=-1)
    o = jnp.einsum('bqk,bkc->bqc', p, v) @ wo
    return o.reshape(B, H, W, C)
```

```python
import functools, math
import jax
import jax.numpy as jnp
from jax import lax
import jax.experimental.pallas as pl
import jax.experimental.pallas.tpu as pltpu

F32 = jnp.float32
BF16 = jnp.bfloat16
WIN = 8
NT = (((1,), (1,)), ((), ()))
L_LO, L_HI, V_HI = 1.0, 2.0 ** 30, 2.0 ** 90


def _tree(op, xs):
    xs = list(xs)
    while len(xs) > 1:
        nxt = [op(xs[i], xs[i + 1]) for i in range(0, len(xs) - 1, 2)]
        if len(xs) % 2:
            nxt.append(xs[-1])
        xs = nxt
    return xs[0]


def _red8(op, s):
    return _tree(op, [s[i * 8:(i + 1) * 8] for i in range(s.shape[0] // 8)])


def build(R=16, U=16, SK=2, UE=4, early=True, fallback=True, PP=1, PB=16, MID=0):
    def pallas_standalone__window_attn_twins__vision_kernel(x, wq, wkv, wo):
        B, H, W, C = x.shape
        nh, nw = H // WIN, W // WIN
        NK = nh * nw
        KC = 8 * nw
        NC = NK // KC
        G = R // UE
        WPG = 8 // G
        assert 8 % G == 0
        scale = C ** (-0.5) * math.log2(math.e)

        def kernel(x_hbm, wq_ref, wkv_ref, wo_ref, o_ref,
                   xv_ref, xs_ref, mt_ref, vt_ref, a_ref, b_ref, acc_ref, l_ref, flag_ref, sems):
            step = pl.program_id(0)

            def copy(w):
                return pltpu.make_async_copy(x_hbm.at[pl.ds(w * WIN, WIN)],
                                             xv_ref.at[pl.ds(w * WIN, WIN)], sems.at[w])

            def pool(w, slot):
                r_i = lax.broadcasted_iota(jnp.int32, (nw, W), 0)
                c_i = lax.broadcasted_iota(jnp.int32, (nw, W), 1)
                pm = jnp.where(c_i // WIN == r_i, 1.0 / (WIN * WIN), 0.0).astype(BF16)
                his, los = [], []
                for rb in range(0, C, PB):
                    hs = None
                    for h in range(0, WIN, 2):
                        t = (xv_ref[w * WIN + h, rb:rb + PB, :].astype(F32)
                             + xv_ref[w * WIN + h + 1, rb:rb + PB, :].astype(F32))
                        hs = t if hs is None else hs + t
                    hi = hs.astype(BF16)
                    his.append(hi)
                    los.append((hs - hi.astype(F32)).astype(BF16))
                hi = jnp.concatenate(his, axis=0)
                lo = jnp.concatenate(los, axis=0)
                xs = (lax.dot_general(pm, hi, NT, preferred_element_type=F32)
                      + lax.dot_general(pm, lo, NT, preferred_element_type=F32))
                xs_ref[pl.ds(pl.multiple_of(slot * nw, 16), nw), :] = xs.astype(BF16)

            def project(j):
                xs = xs_ref[...]
                mt_ref[j] = (jnp.dot(xs, a_ref[...], preferred_element_type=F32) * scale).astype(BF16)
                vt = lax.dot_general(b_ref[...], xs, NT, preferred_element_type=F32)
                vt_ref[j] = vt.astype(BF16)
                vmax = jnp.max(jnp.where(jnp.abs(vt) <= V_HI, 0.0, 1.0))
                flag_ref[0] = jnp.maximum(flag_ref[0], vmax)

            def bad_of(lsum):
                return jnp.where(jnp.logical_and(lsum >= L_LO, lsum <= L_HI), 0.0, 1.0)

            def skewed(items, qk, pv, extra={}):
                for k in range(len(items) + SK):
                    if k < len(items):
                        qk(*items[k])
                    if k >= SK:
                        pv(*items[k - SK])
                    for fn in extra.get(k, []):
                        fn()

            def slow_rows():
                def one(r, _):
                    xt = xv_ref[step * R + r]
                    ss = [jnp.dot(mt_ref[c], xt, preferred_element_type=F32) for c in range(NC)]
                    m = jnp.max(_tree(jnp.maximum, [_red8(jnp.maximum, s) for s in ss]), axis=0, keepdims=True)
                    acc = None; l = None
                    for c in range(NC):
                        p = jnp.exp2(ss[c] - m)
                        lc = _red8(jnp.add, p)
                        y = jnp.dot(vt_ref[c], p.astype(BF16), preferred_element_type=F32)
                        acc = y if acc is None else acc + y
                        l = lc if l is None else l + lc
                    o_ref[r] = (acc / jnp.sum(l, axis=0, keepdims=True)).astype(o_ref.dtype)
                    return 0
                lax.fori_loop(0, R, one, 0)

            def finish(bad):
                if fallback:
                    @pl.when(jnp.maximum(jnp.max(bad), flag_ref[0]) > 0.0)
                    def _():
                        slow_rows()

            def setup():
                for w in range(nh):
                    copy(w).start()
                flag_ref[0] = 0.0
                wkv = wkv_ref[...]
                a_ref[...] = lax.dot_general(wkv[:, :C], wq_ref[...], NT, preferred_element_type=F32).astype(BF16)
                e_r = lax.broadcasted_iota(jnp.int32, (C, C), 0)
                e_c = lax.broadcasted_iota(jnp.int32, (C, C), 1)
                eye = jnp.where(e_r == e_c, 1.0, 0.0).astype(BF16)
                wvo = jnp.dot(wkv[:, C:], wo_ref[...], preferred_element_type=F32).astype(BF16)
                b_ref[...] = lax.dot_general(eye, wvo, NT, preferred_element_type=F32).astype(BF16)

            def main_step():
                def it(i, bad):
                    items = [(u, c) for u in range(U) for c in range(NC)]
                    ps, st = {}, {}
                    bads = [bad]
                    def qk(u, c):
                        xt = xv_ref[step * R + i * U + u]
                        p = jnp.exp2(jnp.dot(mt_ref[c], xt, preferred_element_type=F32))
                        lc = _red8(jnp.add, p)
                        acc, l = st.get(u, (None, None))
                        st[u] = (acc, lc if l is None else l + lc)
                        ps[(u, c)] = p.astype(BF16)
                    def pv(u, c):
                        y = jnp.dot(vt_ref[c], ps.pop((u, c)), preferred_element_type=F32)
                        acc, l = st[u]
                        acc = y if acc is None else acc + y
                        st[u] = (acc, l)
                        if c == NC - 1:
                            lsum = jnp.sum(l, axis=0, keepdims=True)
                            o_ref[i * U + u] = (acc * (1.0 / lsum)).astype(o_ref.dtype)
                            bads.append(bad_of(lsum))
                    skewed(items, qk, pv)
                    return _tree(jnp.maximum, bads)
                bad = lax.fori_loop(0, R // U, it, jnp.zeros((1, W), F32))
                finish(bad)

            def first_pool(w, _):
                copy(w).wait()
                pool(w, w % 8)
                return 0

            if not early:
                @pl.when(step == 0)
                def _():
                    setup()
                    def chunk(j, _):
                        lax.fori_loop(j * 8, j * 8 + 8, first_pool, 0)
                        project(j)
                        return 0
                    lax.fori_loop(0, NC, chunk, 0)
                main_step()
                return

            @pl.when(step == 0)
            def _():
                setup()
                acc_ref[...] = jnp.zeros(acc_ref.shape, F32)
                l_ref[...] = jnp.zeros(l_ref.shape, F32)
                lax.fori_loop(0, 8, first_pool, 0)
                project(0)

                def stage(j, _):
                    def group(g, _):
                        w0 = jnp.minimum(j + 1, NC - 1) * 8 + g * WPG
                        def waits(ts):
                            @pl.when(j < NC - 1)
                            def _():
                                for t in ts:
                                    copy(w0 + t).wait()
                        if not MID:
                            waits(range(WPG))
                        ps = {}
                        def qk(u):
                            r = g * UE + u
                            p = jnp.exp2(jnp.dot(mt_ref[j], xv_ref[r], preferred_element_type=F32))
                            l_ref[r] += _red8(jnp.add, p)
                            ps[u] = p.astype(BF16)
                        def pv(u):
                            r = g * UE + u
                            acc_ref[r] += jnp.dot(vt_ref[j], ps.pop(u), preferred_element_type=F32)
                        extra = {}
                        for t in range(WPG):
                            pos = min(PP + t * max(UE // WPG, 1), UE + SK - 1)
                            if MID:
                                extra.setdefault(max(pos - MID, 0), []).append(functools.partial(waits, [t]))
                            extra.setdefault(pos, []).append(functools.partial(pool, w0 + t, g * WPG + t))
                        skewed([(u,) for u in range(UE)], qk, pv, extra)
                        return 0
                    lax.fori_loop(0, G, group, 0)
                    @pl.when(j < NC - 1)
                    def _():
                        project(j + 1)
                    return 0
                lax.fori_loop(0, NC, stage, 0)

                def fin(r, bad):
                    lsum = jnp.sum(l_ref[r], axis=0, keepdims=True)
                    o_ref[r] = (acc_ref[r] * (1.0 / lsum)).astype(o_ref.dtype)
                    return jnp.maximum(bad, bad_of(lsum))
                finish(lax.fori_loop(0, R, fin, jnp.zeros((1, W), F32), unroll=4))

            @pl.when(step > 0)
            def _():
                main_step()

        xt = x.transpose(0, 1, 3, 2).reshape(H, C, W)
        out = pl.pallas_call(
            kernel,
            grid=(H // R,),
            in_specs=[pl.BlockSpec(memory_space=pl.ANY),
                      pl.BlockSpec((C, C), lambda i: (0, 0)),
                      pl.BlockSpec((C, 2 * C), lambda i: (0, 0)),
                      pl.BlockSpec((C, C), lambda i: (0, 0))],
            out_specs=pl.BlockSpec((R, C, W), lambda i: (i, 0, 0)),
            out_shape=jax.ShapeDtypeStruct((H, C, W), x.dtype),
            scratch_shapes=[pltpu.VMEM((H, C, W), x.dtype),
                            pltpu.VMEM((KC, C), BF16),
                            pltpu.VMEM((NC, KC, C), BF16),
                            pltpu.VMEM((NC, C, KC), BF16),
                            pltpu.VMEM((C, C), BF16),
                            pltpu.VMEM((C, C), BF16),
                            pltpu.VMEM((R, C, W), F32),
                            pltpu.VMEM((R, 8, W), F32),
                            pltpu.SMEM((1,), F32),
                            pltpu.SemaphoreType.DMA((nh,))],
            compiler_params=pltpu.CompilerParams(dimension_semantics=("arbitrary",),
                                                 vmem_limit_bytes=100 * 1024 * 1024),
        )(xt, wq, wkv, wo)
        return out.reshape(B, H, C, W).transpose(0, 1, 3, 2)
    return jax.jit(pallas_standalone__window_attn_twins__vision_kernel)


pallas_standalone__window_attn_twins__vision_kernel = build()
```

```python
import functools
import math

import jax
import jax.numpy as jnp
from jax import lax
import jax.experimental.pallas as pl
import jax.experimental.pallas.tpu as pltpu

F32 = jnp.float32
BF16 = jnp.bfloat16
WIN = 8
LANES = 128
NT = (((1,), (1,)), ((), ()))
TN = (((0,), (0,)), ((), ()))
L_LO, L_HI, V_HI = 1.0, 2.0 ** 30, 2.0 ** 90

R = 16
KEYS_MAIN = 768
SKEW_MAIN = 1
SKEW_A = 2
SKEW_B = 8
POOL_ROWS = 32
OUT_SPLITS = (R - 2, R - 1, R)


def _tree(op, xs):
    xs = list(xs)
    while len(xs) > 1:
        nxt = [op(xs[i], xs[i + 1]) for i in range(0, len(xs) - 1, 2)]
        if len(xs) % 2:
            nxt.append(xs[-1])
        xs = nxt
    return xs[0]


def _red8(op, s):
    return _tree(op, [s[i * 8:(i + 1) * 8] for i in range(s.shape[0] // 8)])


def _skewed(items, qk, pv, skew, tail=()):
    for k in range(len(items) + skew):
        if k < len(items):
            qk(*items[k])
        if k >= skew:
            pv(*items[k - skew])
    for fn in tail:
        fn()


def _kernel(x_hbm, wq_hbm, wkv_hbm, wo_hbm, o_hbm,
            xv_ref, wq_ref, wkv_ref, wo_ref, mt_ref, vt_ref, a_ref, b_ref,
            acc_ref, l_ref, flag_ref, s_ref, ob_ref, wsems, xsems0, xsems, osems):
    H, C, W = xv_ref.shape
    NC, KC, _ = mt_ref.shape
    NK = NC * KC
    NTILE = W // LANES
    CR = WIN * WIN
    KM = KEYS_MAIN if NK % KEYS_MAIN == 0 else KC
    scale = C ** (-0.5) * math.log2(math.e)
    step = pl.program_id(0)
    slot = step % 2

    def wcopies():
        pairs = ((wq_hbm, wq_ref), (wkv_hbm, wkv_ref), (wo_hbm, wo_ref))
        return [pltpu.make_async_copy(s, d, wsems.at[i]) for i, (s, d) in enumerate(pairs)]

    def xcopy_first(w):
        rows = pl.ds(w * WIN, WIN)
        return pltpu.make_async_copy(x_hbm.at[rows], xv_ref.at[rows], xsems0.at[w])

    def xcopy(j):
        rows = pl.ds(j * CR, CR)
        return pltpu.make_async_copy(x_hbm.at[rows], xv_ref.at[rows], xsems.at[j - 1])

    def ocopy(u, n):
        return pltpu.make_async_copy(ob_ref.at[slot, pl.ds(u, n)],
                                     o_hbm.at[pl.ds(step * R + u, n)], osems.at[slot])

    def owait(sl):
        pltpu.make_async_copy(ob_ref.at[sl], ob_ref.at[sl], osems.at[sl]).wait()

    def hsum(w, rb, nrows, t):
        hs = None
        for h in range(0, WIN, 2):
            u = (xv_ref[w * WIN + h, rb:rb + nrows, t * LANES:(t + 1) * LANES].astype(F32)
                 + xv_ref[w * WIN + h + 1, rb:rb + nrows, t * LANES:(t + 1) * LANES].astype(F32))
            hs = u if hs is None else hs + u
        return hs

    def fold_lo(a, bit):
        return a + pltpu.roll(a, LANES - bit, 1)

    def merge_hi(a_folded, b, bit):
        lane = lax.broadcasted_iota(jnp.int32, b.shape, 1)
        return jnp.where((lane & bit) == 0, a_folded, b + pltpu.roll(b, bit, 1))

    def project_tile(j, t, xst):
        mt = lax.dot_general(xst, a_ref[...], TN, preferred_element_type=F32)
        vt = jnp.dot(b_ref[...], xst, preferred_element_type=F32)
        mt_ref[j, t * LANES:(t + 1) * LANES, :] = (mt * scale).astype(BF16)
        vt_ref[j, :, t * LANES:(t + 1) * LANES] = vt.astype(BF16)
        vbad = _red8(jnp.maximum, jnp.where(jnp.abs(vt) <= V_HI, 0.0, 1.0))
        flag_ref[...] = jnp.maximum(flag_ref[...], vbad)

    def pool_tile(j, t):
        pieces = []
        for rb in range(0, C, POOL_ROWS):
            hs = [hsum(j * WIN + i, rb, POOL_ROWS, t) for i in range(WIN)]
            bit = 1
            while len(hs) > 1:
                hs = [merge_hi(fold_lo(hs[k], bit), hs[k + 1], bit) for k in range(0, len(hs), 2)]
                bit *= 2
            pieces.append((hs[0] * (1.0 / CR)).astype(BF16))
        project_tile(j, t, jnp.concatenate(pieces, axis=0))

    def emit_row(u, acc, l):
        lsum = jnp.sum(l, axis=0, keepdims=True)
        ob_ref[slot, u] = (acc * (1.0 / lsum)).astype(ob_ref.dtype)
        return jnp.where(jnp.logical_and(lsum >= L_LO, lsum <= L_HI), 0.0, 1.0)

    def any_unsafe(bads):
        return jnp.maximum(jnp.max(_tree(jnp.maximum, bads)), jnp.max(flag_ref[...]))

    def partial_block(r0, j, skew, emit, tail=()):
        ps, ls, bads = {}, {}, []

        def qk(u):
            p = jnp.exp2(jnp.dot(mt_ref[j], xv_ref[r0 + u], preferred_element_type=F32))
            ls[u] = l_ref[r0 + u] + _red8(jnp.add, p)
            l_ref[r0 + u] = ls[u]
            ps[u] = p.astype(BF16)

        def pv(u):
            acc = acc_ref[r0 + u] + jnp.dot(vt_ref[j], ps.pop(u), preferred_element_type=F32)
            acc_ref[r0 + u] = acc
            if emit:
                bads.append(emit_row(u, acc, ls[u]))

        _skewed([(u,) for u in range(R)], qk, pv, skew, tail)
        return any_unsafe(bads) if emit else None

    def early_step():
        def stage(j, _):
            bad = partial_block(step * R, j, SKEW_A, True)

            @pl.when(j < NC - 1)
            def _():
                xcopy(j + 1).wait()
                partial_block(R, j, SKEW_B, False,
                              [functools.partial(pool_tile, j + 1, t) for t in range(NTILE)])
            return bad

        bad = lax.fori_loop(step * (NC - 1), NC, stage, 0.0)
        ocopy(0, R).start()
        return bad

    def main_step():
        owait(slot)
        ng = NK // KM
        ps, st, bads = {}, {}, []

        def pieces(c):
            out, k = [], c * KM
            while k < (c + 1) * KM:
                hi = min((k // KC + 1) * KC, (c + 1) * KM)
                out.append((k // KC, k % KC, hi - (k // KC) * KC))
                k = hi
            return out

        def qk(u, c):
            mt = jnp.concatenate([mt_ref[j, lo:hi, :] for j, lo, hi in pieces(c)], axis=0)
            p = jnp.exp2(jnp.dot(mt, xv_ref[step * R + u], preferred_element_type=F32))
            lc = _red8(jnp.add, p)
            st[u] = (None, lc) if c == 0 else (st[u][0], st[u][1] + lc)
            ps[(u, c)] = p.astype(BF16)

        def pv(u, c):
            vt = jnp.concatenate([vt_ref[j, :, lo:hi] for j, lo, hi in pieces(c)], axis=1)
            y = jnp.dot(vt, ps.pop((u, c)), preferred_element_type=F32)
            acc, l = st[u]
            acc = y if acc is None else acc + y
            st[u] = (acc, l)
            if c == ng - 1:
                bads.append(emit_row(u, acc, l))
                if u + 1 in OUT_SPLITS:
                    prev = max([0] + [e for e in OUT_SPLITS if e < u + 1])
                    ocopy(prev, u + 1 - prev).start()

        _skewed([(u, c) for u in range(R) for c in range(ng)], qk, pv, SKEW_MAIN)
        return any_unsafe(bads)

    def true_max_rows():
        def one(r, _):
            def qk(c, m):
                s = jnp.dot(mt_ref[c], xv_ref[step * R + r], preferred_element_type=F32)
                s_ref[c] = s
                return jnp.maximum(m, _red8(jnp.maximum, s))

            m = lax.fori_loop(0, NC, qk, jnp.full((8, W), -jnp.inf, F32))
            m = jnp.max(m, axis=0, keepdims=True)

            def pv(c, carry):
                acc, l = carry
                p = jnp.exp2(s_ref[c] - m)
                return (acc + jnp.dot(vt_ref[c], p.astype(BF16), preferred_element_type=F32),
                        l + _red8(jnp.add, p))

            acc, l = lax.fori_loop(0, NC, pv, (jnp.zeros((C, W), F32), jnp.zeros((8, W), F32)))
            ob_ref[slot, r] = (acc / jnp.sum(l, axis=0, keepdims=True)).astype(ob_ref.dtype)
            return 0

        lax.fori_loop(0, R, one, 0)

    @pl.when(step == 0)
    def _():
        for cp in wcopies():
            cp.start()
        for w in range(WIN):
            xcopy_first(w).start(priority=1)
        for j in range(1, NC):
            xcopy(j).start(priority=1)
        flag_ref[...] = jnp.zeros(flag_ref.shape, F32)

        def zero(r, _):
            acc_ref[r] = jnp.zeros((C, W), F32)
            l_ref[r] = jnp.zeros((8, W), F32)
            return 0

        lax.fori_loop(0, 2 * R, zero, 0)
        for cp in wcopies():
            cp.wait()
        wkv = wkv_ref[...]
        a_ref[...] = lax.dot_general(wkv[:, :C], wq_ref[...], NT,
                                     preferred_element_type=F32).astype(BF16)
        b_ref[...] = jnp.dot(wkv[:, C:], wo_ref[...], preferred_element_type=F32).T.astype(BF16)
        stack = []
        for i in range(WIN):
            xcopy_first(i).wait()
            cur = [hsum(i, 0, C, t) for t in range(NTILE)]
            bit = 1
            while i & bit:
                cur = [merge_hi(a, b, bit) for a, b in zip(stack.pop(), cur)]
                bit *= 2
            stack.append([fold_lo(a, bit) for a in cur] if i < WIN - 1 else cur)
        for t in range(NTILE):
            project_tile(0, t, (stack[0][t] * (1.0 / CR)).astype(BF16))

    unsafe = lax.cond(step < 2, early_step, main_step)

    @pl.when(unsafe > 0.0)
    def _():
        owait(slot)
        true_max_rows()
        ocopy(0, R).start()

    @pl.when(step == pl.num_programs(0) - 1)
    def _():
        owait(1 - slot)
        owait(slot)


@jax.jit
def pallas_standalone__window_attn_twins__vision_kernel(
    x: jax.Array,
    wq: jax.Array,
    wkv: jax.Array,
    wo: jax.Array,
):
    B, H, W, C = x.shape
    assert B == 1 and H % (WIN * WIN) == 0 and H >= 2 * WIN * WIN and W % LANES == 0
    assert C % POOL_ROWS == 0 and 2 * R <= WIN * WIN
    nc = H // (WIN * WIN)
    xt = x.transpose(0, 1, 3, 2).reshape(H, C, W)
    out = pl.pallas_call(
        _kernel,
        grid=(H // R,),
        in_specs=[pl.BlockSpec(memory_space=pl.ANY)] * 4,
        out_specs=pl.BlockSpec(memory_space=pl.ANY),
        out_shape=jax.ShapeDtypeStruct((H, C, W), x.dtype),
        scratch_shapes=[
            pltpu.VMEM((H, C, W), x.dtype),
            pltpu.VMEM((C, C), wq.dtype),
            pltpu.VMEM((C, 2 * C), wkv.dtype),
            pltpu.VMEM((C, C), wo.dtype),
            pltpu.VMEM((nc, W, C), BF16),
            pltpu.VMEM((nc, C, W), BF16),
            pltpu.VMEM((C, C), BF16),
            pltpu.VMEM((C, C), BF16),
            pltpu.VMEM((2 * R, C, W), F32),
            pltpu.VMEM((2 * R, 8, W), F32),
            pltpu.VMEM((8, LANES), F32),
            pltpu.VMEM((nc, W, W), F32),
            pltpu.VMEM((2, R, C, W), x.dtype),
            pltpu.SemaphoreType.DMA((3,)),
            pltpu.SemaphoreType.DMA((WIN,)),
            pltpu.SemaphoreType.DMA((nc - 1,)),
            pltpu.SemaphoreType.DMA((2,)),
        ],
        compiler_params=pltpu.CompilerParams(
            dimension_semantics=("arbitrary",),
            vmem_limit_bytes=100 * 1024 * 1024,
        ),
    )(xt, wq, wkv, wo)
    return out.reshape(B, H, C, W).transpose(0, 1, 3, 2)
```

```python
import math

import jax
import jax.numpy as jnp
from jax import lax
import jax.experimental.pallas as pl
import jax.experimental.pallas.tpu as pltpu

F32 = jnp.float32
BF16 = jnp.bfloat16
U32 = jnp.uint32
WIN = 8
LANES = 128
NT = (((1,), (1,)), ((), ()))
TN = (((0,), (0,)), ((), ()))
L_LO, L_HI, V_HI = 1.0, 2.0 ** 30, 2.0 ** 90

R = 16
KEYS_MAIN = 768
SKEW_MAIN = 1
SKEW_A = 2
SKEW_B = R
POOL_ROWS = 32
OUT_SPLITS = (R - 2, R - 1, R)


def _tree(op, xs):
    xs = list(xs)
    while len(xs) > 1:
        nxt = [op(xs[i], xs[i + 1]) for i in range(0, len(xs) - 1, 2)]
        if len(xs) % 2:
            nxt.append(xs[-1])
        xs = nxt
    return xs[0]


def _red8(op, s):
    return _tree(op, [s[i * 8:(i + 1) * 8] for i in range(s.shape[0] // 8)])


def _skewed(items, qk, pv, skew, tail=()):
    n = len(items) + skew
    for k in range(n):
        if k < len(items):
            qk(*items[k])
        if k >= skew:
            pv(*items[k - skew])
        if k >= n - len(tail):
            tail[k - (n - len(tail))]()


def _blk(i, size):
    return pl.ds(i * size if isinstance(i, int) else pl.multiple_of(i * size, size), size)


def _kernel(x_hbm, wq_hbm, wkv_hbm, wo_hbm, o_hbm,
            xv_ref, wq_ref, wkv_ref, wo_ref, mt_ref, vt_ref, a_ref, b_ref,
            acc_ref, l_ref, flag_ref, s_ref, ob_ref, wsems, xsems0, xsems, osems):
    H, C, W = xv_ref.shape
    NC, _, KC = vt_ref.shape
    NK = NC * KC
    NTILE = W // LANES
    CR = WIN * WIN
    KM = KEYS_MAIN if NK % KEYS_MAIN == 0 and KEYS_MAIN % KC == 0 else KC
    scale = C ** (-0.5) * math.log2(math.e)
    step = pl.program_id(0)
    slot = step % 2

    def wcopies():
        pairs = ((wq_hbm, wq_ref), (wkv_hbm, wkv_ref), (wo_hbm, wo_ref))
        return [pltpu.make_async_copy(s, d, wsems.at[i]) for i, (s, d) in enumerate(pairs)]

    def xcopy_first(w):
        rows = pl.ds(w * WIN, WIN)
        return pltpu.make_async_copy(x_hbm.at[rows], xv_ref.at[rows], xsems0.at[w])

    def xcopy(j):
        rows = pl.ds(j * CR, CR)
        return pltpu.make_async_copy(x_hbm.at[rows], xv_ref.at[rows], xsems.at[j - 2])

    def ocopy(u, n):
        return pltpu.make_async_copy(ob_ref.at[slot, pl.ds(u, n)],
                                     o_hbm.at[pl.ds(step * R + u, n)], osems.at[slot])

    def owait(sl):
        pltpu.make_async_copy(ob_ref.at[sl], ob_ref.at[sl], osems.at[sl]).wait()

    def hsum(w, rb, nrows, t):
        hs = None
        for h in range(0, WIN, 2):
            u = (xv_ref[w * WIN + h, rb:rb + nrows, _blk(t, LANES)].astype(F32)
                 + xv_ref[w * WIN + h + 1, rb:rb + nrows, _blk(t, LANES)].astype(F32))
            hs = u if hs is None else hs + u
        return hs

    def fold_lo(a, bit):
        return a + pltpu.roll(a, LANES - bit, 1)

    def merge_hi(a_folded, b, bit):
        lane = lax.broadcasted_iota(jnp.int32, b.shape, 1)
        return jnp.where((lane & bit) == 0, a_folded, b + pltpu.roll(b, bit, 1))

    def project(xst):
        mt = lax.dot_general(xst, a_ref[...], TN, preferred_element_type=F32)
        vt = jnp.dot(b_ref[...], xst, preferred_element_type=F32)
        vbad = _red8(jnp.maximum, jnp.where(jnp.abs(vt) <= V_HI, 0.0, 1.0))
        return (mt * scale).astype(BF16), vt.astype(BF16), vbad

    def pool(srcs):
        pieces = []
        for rb in range(0, C, POOL_ROWS):
            hs = [hsum(w, rb, POOL_ROWS, t) for w, t in srcs]
            bit = 1
            while len(hs) > 1:
                hs = [merge_hi(fold_lo(hs[k], bit), hs[k + 1], bit) for k in range(0, len(hs), 2)]
                bit *= 2
            pieces.append((hs[0] * (1.0 / CR)).astype(BF16))
        return project(jnp.concatenate(pieces, axis=0))

    def store_keys(j, t, vals):
        mt, vt, vbad = vals
        mt_ref[j, _blk(t, LANES // 2), :] = pltpu.bitcast(mt, U32)
        vt_ref[j, :, _blk(t, LANES)] = pltpu.bitcast(vt, U32)
        flag_ref[...] = jnp.maximum(flag_ref[...], vbad)

    def keys_m(j, t=None):
        v = mt_ref[j] if t is None else mt_ref[j, _blk(t, LANES // 2), :]
        return pltpu.bitcast(v, BF16)

    def keys_v(j, t=None):
        v = vt_ref[j] if t is None else vt_ref[j, :, _blk(t, LANES)]
        return pltpu.bitcast(v, BF16)

    def emit_row(u, acc, l):
        lsum = jnp.sum(l, axis=0, keepdims=True)
        ob_ref[slot, u] = (acc * (1.0 / lsum)).astype(ob_ref.dtype)
        return jnp.where(jnp.logical_and(lsum >= L_LO, lsum <= L_HI), 0.0, 1.0)

    def any_unsafe(bads):
        return jnp.maximum(jnp.max(_tree(jnp.maximum, bads)), jnp.max(flag_ref[...]))

    def partial_block(r0, j, t=None, new_keys=()):
        ps, ls, bads, built = {}, {}, [], []

        def qk(u):
            p = jnp.exp2(jnp.dot(keys_m(j, t), xv_ref[r0 + u], preferred_element_type=F32))
            ls[u] = l_ref[r0 + u] + _red8(jnp.add, p)
            l_ref[r0 + u] = ls[u]
            ps[u] = p.astype(BF16)

        def pv(u):
            acc = acc_ref[r0 + u] + jnp.dot(keys_v(j, t), ps.pop(u), preferred_element_type=F32)
            acc_ref[r0 + u] = acc
            if not new_keys:
                bads.append(emit_row(u, acc, ls[u]))

        _skewed([(u,) for u in range(R)], qk, pv, SKEW_B if new_keys else SKEW_A,
                [lambda srcs=srcs: built.append(pool(srcs)) for _, _, srcs in new_keys])
        for (jn, tn, _), vals in zip(new_keys, built):
            store_keys(jn, tn, vals)
        return None if new_keys else any_unsafe(bads)

    def early_step():
        def stage(j, _):
            bad = partial_block(step * R, j)

            @pl.when(j < NC - 1)
            def _():
                xcopy(j + 1).wait()
                partial_block(R, j, None,
                              [(j + 1, t, [((j + 1) * WIN + i, t) for i in range(WIN)])
                               for t in range(NTILE)])
            return bad

        bad = lax.fori_loop(1 + step * (NC - 2), NC, stage, 0.0)
        ocopy(0, R).start()
        return bad

    def main_step():
        owait(slot)
        cpi = KM // KC
        ng = NC // cpi
        ps, st, bads = {}, {}, []

        def qk(u, c):
            mt = jnp.concatenate([keys_m(c * cpi + i) for i in range(cpi)], axis=0)
            p = jnp.exp2(jnp.dot(mt, xv_ref[step * R + u], preferred_element_type=F32))
            lc = _red8(jnp.add, p)
            st[u] = (None, lc) if c == 0 else (st[u][0], st[u][1] + lc)
            ps[(u, c)] = p.astype(BF16)

        def pv(u, c):
            vt = jnp.concatenate([keys_v(c * cpi + i) for i in range(cpi)], axis=1)
            y = jnp.dot(vt, ps.pop((u, c)), preferred_element_type=F32)
            acc, l = st[u]
            acc = y if acc is None else acc + y
            st[u] = (acc, l)
            if c == ng - 1:
                bads.append(emit_row(u, acc, l))
                if u + 1 in OUT_SPLITS:
                    prev = max([0] + [e for e in OUT_SPLITS if e < u + 1])
                    ocopy(prev, u + 1 - prev).start()

        _skewed([(u, c) for u in range(R) for c in range(ng)], qk, pv, SKEW_MAIN)
        return any_unsafe(bads)

    def true_max_rows():
        def one(r, _):
            def qk(c, m):
                s = jnp.dot(keys_m(c), xv_ref[step * R + r], preferred_element_type=F32)
                s_ref[c] = s
                return jnp.maximum(m, _red8(jnp.maximum, s))

            m = lax.fori_loop(0, NC, qk, jnp.full((8, W), -jnp.inf, F32))
            m = jnp.max(m, axis=0, keepdims=True)

            def pv(c, carry):
                acc, l = carry
                p = jnp.exp2(s_ref[c] - m)
                return (acc + jnp.dot(keys_v(c), p.astype(BF16), preferred_element_type=F32),
                        l + _red8(jnp.add, p))

            acc, l = lax.fori_loop(0, NC, pv, (jnp.zeros((C, W), F32), jnp.zeros((8, W), F32)))
            ob_ref[slot, r] = (acc / jnp.sum(l, axis=0, keepdims=True)).astype(ob_ref.dtype)
            return 0

        lax.fori_loop(0, R, one, 0)

    @pl.when(step == 0)
    def _():
        for cp in wcopies():
            cp.start()
        for w in range(2 * WIN):
            xcopy_first(w).start(priority=1)
        for j in range(2, NC):
            xcopy(j).start(priority=1)
        flag_ref[...] = jnp.zeros(flag_ref.shape, F32)

        def zero(r, _):
            acc_ref[r] = jnp.zeros((C, W), F32)
            l_ref[r] = jnp.zeros((8, W), F32)
            return 0

        lax.fori_loop(0, 2 * R, zero, 0)
        for cp in wcopies():
            cp.wait()
        wkv = wkv_ref[...]
        a_ref[...] = lax.dot_general(wkv[:, :C], wq_ref[...], NT,
                                     preferred_element_type=F32).astype(BF16)
        b_ref[...] = jnp.dot(wkv[:, C:], wo_ref[...], preferred_element_type=F32).T.astype(BF16)
        stack = []
        for q in range(WIN):
            if q % NTILE == 0:
                xcopy_first(q // NTILE).wait()
            cur = hsum(q // NTILE, 0, C, q % NTILE)
            bit = 1
            while q & bit:
                cur = merge_hi(stack.pop(), cur, bit)
                bit *= 2
            stack.append(fold_lo(cur, bit) if q < WIN - 1 else cur)
        store_keys(0, 0, project((stack[0] * (1.0 / CR)).astype(BF16)))

        def last_row(n):
            return jnp.maximum((WIN * n + WIN - 1) // NTILE, ((n % 2 + 1) * R - 1) // WIN)

        def first_chunk(n, done):
            need = jnp.maximum(done, last_row(n) + 1)

            def wait_row(w, _):
                xcopy_first(w).wait()
                return 0

            lax.fori_loop(done, need, wait_row, 0)
            partial_block((n % 2) * R, 0, n // 2,
                          [(n // NTILE, n % NTILE,
                            [((WIN * n + i) // NTILE, (WIN * n + i) % NTILE) for i in range(WIN)])])
            return need

        lax.fori_loop(0, 2 * NTILE, first_chunk, (WIN - 1) // NTILE + 1)

    unsafe = lax.cond(step < 2, early_step, main_step)

    @pl.when(unsafe > 0.0)
    def _():
        owait(slot)
        true_max_rows()
        ocopy(0, R).start()

    @pl.when(step == pl.num_programs(0) - 1)
    def _():
        owait(1 - slot)
        owait(slot)


@jax.jit
def pallas_standalone__window_attn_twins__vision_kernel(
    x: jax.Array,
    wq: jax.Array,
    wkv: jax.Array,
    wo: jax.Array,
):
    B, H, W, C = x.shape
    assert B == 1 and H % (WIN * WIN) == 0 and H >= 3 * WIN * WIN and W % LANES == 0
    assert C % POOL_ROWS == 0 and 2 * R <= WIN * WIN
    nc = H // (WIN * WIN)
    xt = x.transpose(0, 1, 3, 2).reshape(H, C, W)
    out = pl.pallas_call(
        _kernel,
        grid=(H // R,),
        in_specs=[pl.BlockSpec(memory_space=pl.ANY)] * 4,
        out_specs=pl.BlockSpec(memory_space=pl.ANY),
        out_shape=jax.ShapeDtypeStruct((H, C, W), x.dtype),
        scratch_shapes=[
            pltpu.VMEM((H, C, W), x.dtype),
            pltpu.VMEM((C, C), wq.dtype),
            pltpu.VMEM((C, 2 * C), wkv.dtype),
            pltpu.VMEM((C, C), wo.dtype),
            pltpu.VMEM((nc, W // 2, C), U32),
            pltpu.VMEM((nc, C // 2, W), U32),
            pltpu.VMEM((C, C), BF16),
            pltpu.VMEM((C, C), BF16),
            pltpu.VMEM((2 * R, C, W), F32),
            pltpu.VMEM((2 * R, 8, W), F32),
            pltpu.VMEM((8, LANES), F32),
            pltpu.VMEM((nc, W, W), F32),
            pltpu.VMEM((2, R, C, W), x.dtype),
            pltpu.SemaphoreType.DMA((3,)),
            pltpu.SemaphoreType.DMA((2 * WIN,)),
            pltpu.SemaphoreType.DMA((nc - 2,)),
            pltpu.SemaphoreType.DMA((2,)),
        ],
        compiler_params=pltpu.CompilerParams(
            dimension_semantics=("arbitrary",),
            vmem_limit_bytes=100 * 1024 * 1024,
            disable_bounds_checks=True,
            disable_semaphore_checks=True,
        ),
    )(xt, wq, wkv, wo)
    return out.reshape(B, H, C, W).transpose(0, 1, 3, 2)
```

```python
import math

import jax
import jax.numpy as jnp
from jax import lax
import jax.experimental.pallas as pl
import jax.experimental.pallas.tpu as pltpu

F32 = jnp.float32
BF16 = jnp.bfloat16
U32 = jnp.uint32
WIN = 8
LANES = 128
NT = (((1,), (1,)), ((), ()))
TN = (((0,), (0,)), ((), ()))
L_LO, L_HI, V_HI = 1.0, 2.0 ** 30, 2.0 ** 90

RE = 17
RM = 14
NV = 64
SKEW_MAIN = 12
SKEW_A = 2
TIES = 4
GROUP = 2
RING = 9
CH_BLK = 32
POOL_ROWS = 48
OUT_SPLITS = (RM - 2, RM - 1, RM)


def _tree(op, xs):
    xs = list(xs)
    while len(xs) > 1:
        nxt = [op(xs[i], xs[i + 1]) for i in range(0, len(xs) - 1, 2)]
        if len(xs) % 2:
            nxt.append(xs[-1])
        xs = nxt
    return xs[0]


def _red8(reduce, s):
    n, lanes = s.shape[0] // 8, s.shape[1]
    while n > 1:
        r = 2 if n % 2 == 0 else n
        s = reduce(s.reshape(n // r, r, 8, lanes), axis=1)
        n //= r
    return s.reshape(8, lanes)


def _skewed(n, qk, pv, skew, tail=()):
    m = n + skew
    for k in range(m):
        if k < n:
            qk(k)
        if k >= skew:
            pv(k - skew)
        if k >= m - len(tail):
            tail[k - (m - len(tail))]()


def _blk(i, size):
    return pl.ds(i * size if isinstance(i, int) else pl.multiple_of(i * size, size), size)


def _stager(bufs, i):
    spare = bufs[0].shape[0] - 16
    fence = pl.ds(pl.multiple_of((lax.shift_right_logical(i, 20) + 1) * spare, 16), 16)
    zeros = jnp.zeros((16, LANES), BF16)

    def put(k, p):
        bufs[k % len(bufs)][0:p.shape[0], 0:p.shape[1]] = p.astype(BF16)
        bufs[k % len(bufs)][fence, 0:LANES] = zeros

    def get(k, rows, cols):
        return bufs[k % len(bufs)][0:rows, 0:cols]

    return put, get


def _kernel(x_hbm, wq_hbm, wkv_hbm, wo_hbm, o_hbm,
            xv_ref, wq_ref, wkv_ref, wo_ref, mt_ref, vt_ref, a_ref, b_ref,
            acc_ref, l_ref, flag_ref, s_ref, oe_ref, ob_ref, mb_ref, sv_ref, z_ref,
            wsems, xsems0, xsems, osems, *stage_refs):
    H, C, W = xv_ref.shape
    NC = vt_ref.shape[0]
    NTILE = W // LANES
    CR = WIN * WIN
    NB = flag_ref.shape[0] - 1
    G = NV // 16
    V0 = (LANES - NV) // 2
    scale = C ** (-0.5) * math.log2(math.e)
    stage_refs = [r.bitcast(BF16) for r in stage_refs]
    p_refs, pe_refs = stage_refs[:RING], stage_refs[RING:]

    def wcopies():
        pairs = ((wq_hbm, wq_ref), (wkv_hbm, wkv_ref), (wo_hbm, wo_ref))
        return [pltpu.make_async_copy(s, d, wsems.at[i]) for i, (s, d) in enumerate(pairs)]

    def xcopy_first(w):
        rows = pl.ds(w * WIN, WIN)
        return pltpu.make_async_copy(x_hbm.at[rows], xv_ref.at[rows], xsems0.at[w])

    def xcopy(j):
        rows = pl.ds(j * CR, CR)
        return pltpu.make_async_copy(x_hbm.at[rows], xv_ref.at[rows], xsems.at[j - 2])

    def ecopy():
        return pltpu.make_async_copy(oe_ref, o_hbm.at[pl.ds(0, 2 * RE)], osems.at[2])

    def owait(sl):
        pltpu.make_async_copy(ob_ref.at[sl], ob_ref.at[sl], osems.at[sl]).wait()

    def hsum(w, rb, nrows, t):
        hs = None
        for h in range(0, WIN, 2):
            u = (xv_ref[w * WIN + h, rb:rb + nrows, _blk(t, LANES)].astype(F32)
                 + xv_ref[w * WIN + h + 1, rb:rb + nrows, _blk(t, LANES)].astype(F32))
            hs = u if hs is None else hs + u
        return hs

    def fold_lo(a, bit):
        return a + pltpu.roll(a, LANES - bit, 1)

    def merge_hi(a_folded, b, bit):
        lane = lax.broadcasted_iota(jnp.int32, b.shape, 1)
        return jnp.where((lane & bit) == 0, a_folded, b + pltpu.roll(b, bit, 1))

    def project(xst):
        mt = lax.dot_general(xst, a_ref[...], TN, preferred_element_type=F32)
        vt = jnp.dot(b_ref[...], xst, preferred_element_type=F32)
        vbad = _red8(jnp.max, jnp.where(jnp.abs(vt) <= V_HI, 0.0, 1.0))
        return (mt * scale).astype(BF16), vt.astype(BF16), vbad

    def pool(srcs):
        pieces = []
        for rb in range(0, C, POOL_ROWS):
            hs = [hsum(w, rb, POOL_ROWS, t) for w, t in srcs]
            bit = 1
            while len(hs) > 1:
                hs = [merge_hi(fold_lo(hs[k], bit), hs[k + 1], bit) for k in range(0, len(hs), 2)]
                bit *= 2
            pieces.append((hs[0] * (1.0 / CR)).astype(BF16))
        return project(jnp.concatenate(pieces, axis=0))

    def store_keys(j, t, vals):
        mt, vt, vbad = vals
        mt_ref[j, _blk(t, LANES // 2), :] = pltpu.bitcast(mt, U32)
        vt_ref[j, :, _blk(t, LANES)] = pltpu.bitcast(vt, U32)
        flag_ref[NB] = jnp.maximum(flag_ref[NB], vbad)

    def keys_m(j, t=None):
        v = mt_ref[j] if t is None else mt_ref[j, _blk(t, LANES // 2), :]
        return pltpu.bitcast(v, BF16)

    def keys_v(j, t=None):
        v = vt_ref[j] if t is None else vt_ref[j, :, _blk(t, LANES)]
        return pltpu.bitcast(v, BF16)

    def spread_keys(g):
        m = mt_ref[0, pl.ds(pl.multiple_of(V0 + g * 8, 8), 8), :]
        m = pltpu.bitcast(m, BF16).astype(F32)
        for ch in range(C):
            mb_ref[ch, _blk(g, 16), :] = jnp.broadcast_to(m[:, ch:ch + 1], (16, LANES))

    def finish(acc, l):
        lsum = jnp.sum(l, axis=0, keepdims=True)
        bad = jnp.where(jnp.logical_and(lsum >= L_LO, lsum <= L_HI), 0.0, 1.0)
        return ((acc * (1.0 / lsum)).astype(BF16),
                [bad[:, i:i + LANES] for i in range(0, bad.shape[1], LANES)])

    def set_flag(b, bads):
        flag_ref[b] = jnp.broadcast_to(_tree(jnp.maximum, bads), (8, LANES))

    def early_block(half, j, t=None, new_keys=(), i=None):
        r0 = half * RE
        ps, ls, bads, built = {}, {}, [], []
        if new_keys:
            put, get = _stager(pe_refs, i)

        def qk(u):
            p = jnp.exp2(jnp.dot(keys_m(j, t), xv_ref[r0 + u], preferred_element_type=F32))
            if new_keys:
                put(u, p)
            ls[u] = l_ref[r0 + u] + _red8(jnp.sum, p)
            l_ref[r0 + u] = ls[u]
            ps[u] = p

        def pv(u):
            p = ps.pop(u)
            p = get(u, *p.shape) if new_keys else p.astype(BF16)
            acc = acc_ref[r0 + u] + jnp.dot(keys_v(j, t), p, preferred_element_type=F32)
            acc_ref[r0 + u] = acc
            if not new_keys:
                oe_ref[r0 + u], bad = finish(acc, ls[u])
                bads.extend(bad)

        _skewed(RE, qk, pv, RE if new_keys else SKEW_A,
                [lambda srcs=srcs: built.append(pool(srcs)) for _, _, srcs in new_keys])
        for (jn, tn, _), vals in zip(new_keys, built):
            store_keys(jn, tn, vals)
        if bads:
            set_flag(half, bads)

    def main_block(b, _):
        slot = lax.rem(b, 2)
        row0 = 2 * RE + b * RM

        @pl.when(b >= 2)
        def _():
            owait(slot)

        put, get = _stager(p_refs, b)
        order = list(range(1, NC * NTILE)) + [0]
        items = [(u, t, kt) for u in range(RM) for t in range(NTILE) for kt in order]
        steps = [(u, g, ch) for u in range(1, RM + 1) for g in range(2) for ch in range(C)]
        work = {}
        for n, stp in enumerate(steps):
            work.setdefault((2 * n + 1) * len(items) * TIES // (2 * len(steps)), []).append(stp)
        never = jnp.broadcast_to((z_ref[:, :C] != 0)[None], (TIES, 8, C))
        sv, ops, qops, vops, st, pend, bads, last = {}, {}, {}, {}, {}, [], [], [0, None]

        def vpu(n):
            for u, g, ch in work.get(n, ()):
                key = (u, g, ch // CH_BLK)
                if key not in ops:
                    row = row0 + u if u < RM else jnp.minimum(row0 + u, H - 1)
                    xb = xv_ref[row, _blk(ch // CH_BLK, CH_BLK), :].astype(F32)
                    ops[key] = (jnp.stack([xb[:, t * LANES:(t + 1) * LANES] for t in range(NTILE)]),
                                mb_ref[_blk(ch // CH_BLK, CH_BLK), _blk(g, G * 8), :])
                xb, mb = ops[key]
                c = ch % CH_BLK
                term = mb[c:c + 1] * xb[:, c:c + 1, :]
                sv[(u, g)] = term if ch == 0 else sv[(u, g)] + term
            if n in work:
                last[0] = (last[0] + 1) % G
                last[1] = sv[(u, g)][NTILE - 1:, last[0] * 8:last[0] * 8 + 8, :C]
            return last[1]

        def qk(k):
            u, t, kt = items[k]
            if (u, t) not in qops:
                qops[(u, t)] = (xv_ref[row0 + u, :, _blk(t, LANES)], mt_ref[...])
            xt, mt = qops[(u, t)]
            rows = (LANES - NV if kt == 0 else LANES) // 2
            j, lo = kt // NTILE, (kt % NTILE) * (LANES // 2)
            mt = mt[j:j + 1, lo:lo + rows].reshape(TIES, rows // TIES, C)
            tie = pltpu.bitcast(jnp.concatenate([vpu(k * TIES + a) for a in range(TIES)], axis=0), U32)
            if rows == 8 * TIES:
                mt = lax.select(never, tie, mt)
            else:
                mt = jnp.concatenate([mt[:, :-8], lax.select(never, tie, mt[:, -8:])], axis=1)
            s = jnp.dot(pltpu.bitcast(mt.reshape(rows, C), BF16), xt, preferred_element_type=F32)
            pend.append(s)
            if kt == 0:
                pend.extend([sv_ref[:, _blk(t, LANES)]] if u == 0 else [sv[(u, 0)][t], sv[(u, 1)][t]])
            if k % GROUP == GROUP - 1:
                p = jnp.exp2(jnp.concatenate(pend, axis=0))
                del pend[:]
                put(k // GROUP, p)
                lc = _red8(jnp.sum, p)
                acc, l = st.get((u, t), (None, None))
                st[(u, t)] = (acc, lc if l is None else l + lc)

        def pv(k):
            u, t, kt = items[k]
            if (u, t) not in vops:
                vops[(u, t)] = pltpu.bitcast(vt_ref[...], BF16)
            if k % GROUP == 0:
                vops["p"] = get(k // GROUP, GROUP * LANES, LANES)
            vt = vops[(u, t)][kt // NTILE, :, (kt % NTILE) * LANES:(kt % NTILE + 1) * LANES]
            p = vops["p"][(k % GROUP) * LANES:(k % GROUP + 1) * LANES]
            y = jnp.dot(vt, p, preferred_element_type=F32)
            acc, l = st[(u, t)]
            acc = y if acc is None else acc + y
            st[(u, t)] = (acc, l)
            if kt == 0:
                ob_ref[slot, u, :, _blk(t, LANES)], bad = finish(acc, l)
                bads.extend(bad)
                if t == NTILE - 1 and u + 1 in OUT_SPLITS:
                    lo = max([0] + [e for e in OUT_SPLITS if e < u + 1])
                    pltpu.make_async_copy(ob_ref.at[slot, pl.ds(lo, u + 1 - lo)],
                                          o_hbm.at[pl.ds(row0 + lo, u + 1 - lo)],
                                          osems.at[slot]).start()

        _skewed(len(items), qk, pv, SKEW_MAIN)
        sv_ref[...] = jnp.concatenate(
            [jnp.concatenate([sv[(RM, g)][t] for t in range(NTILE)], axis=1) for g in range(2)], axis=0)
        set_flag(2 + b, bads)
        return 0

    def true_max_row(r, _):
        def tile(t, _):
            lanes = _blk(t, LANES)

            def qk(c, m):
                s = jnp.dot(keys_m(c), xv_ref[r, :, lanes], preferred_element_type=F32)
                s_ref[c] = s
                return jnp.maximum(m, _red8(jnp.max, s))

            m = lax.fori_loop(0, NC, qk, jnp.full((8, LANES), -jnp.inf, F32))
            m = jnp.max(m, axis=0, keepdims=True)

            def pv(c, carry):
                acc, l = carry
                p = jnp.exp2(s_ref[c] - m)
                return (acc + jnp.dot(keys_v(c), p.astype(BF16), preferred_element_type=F32),
                        l + _red8(jnp.sum, p))

            acc, l = lax.fori_loop(0, NC, pv,
                                   (jnp.zeros((C, LANES), F32), jnp.zeros((8, LANES), F32)))
            oe_ref[0, :, lanes] = (acc / jnp.sum(l, axis=0, keepdims=True)).astype(BF16)
            return 0

        lax.fori_loop(0, NTILE, tile, 0)
        cp = pltpu.make_async_copy(oe_ref.at[0], o_hbm.at[r], osems.at[2])
        cp.start()
        cp.wait()
        return 0

    for cp in wcopies():
        cp.start()
    for w in range(2 * WIN):
        xcopy_first(w).start(priority=1)
    for j in range(2, NC):
        xcopy(j).start(priority=1)
    flag_ref[...] = jnp.zeros(flag_ref.shape, F32)
    z_ref[...] = jnp.zeros(z_ref.shape, U32)

    def zero(r, _):
        acc_ref[r] = jnp.zeros((C, W), F32)
        l_ref[r] = jnp.zeros((8, W), F32)
        return 0

    lax.fori_loop(0, 2 * RE, zero, 0)
    for cp in wcopies():
        cp.wait()
    wkv = wkv_ref[...]
    a_ref[...] = lax.dot_general(wkv[:, :C], wq_ref[...], NT, preferred_element_type=F32).astype(BF16)
    b_ref[...] = jnp.dot(wkv[:, C:], wo_ref[...], preferred_element_type=F32).T.astype(BF16)

    stack = []
    for q in range(WIN):
        if q % NTILE == 0:
            xcopy_first(q // NTILE).wait()
        cur = hsum(q // NTILE, 0, C, q % NTILE)
        bit = 1
        while q & bit:
            cur = merge_hi(stack.pop(), cur, bit)
            bit *= 2
        stack.append(fold_lo(cur, bit) if q < WIN - 1 else cur)
    store_keys(0, 0, project((stack[0] * (1.0 / CR)).astype(BF16)))

    def first_chunk(n, done):
        half = lax.rem(n, 2)
        last = jnp.maximum(lax.div(WIN * n + WIN - 1, NTILE),
                           lax.div((half + 1) * RE - 1, WIN))
        need = jnp.maximum(done, last + 1)

        def wait_row(w, _):
            xcopy_first(w).wait()
            return 0

        lax.fori_loop(done, need, wait_row, 0)
        srcs = [(lax.div(WIN * n + i, NTILE), lax.rem(WIN * n + i, NTILE)) for i in range(WIN)]
        early_block(half, 0, lax.div(n, 2), [(lax.div(n, NTILE), lax.rem(n, NTILE), srcs)], n)
        return need

    lax.fori_loop(0, 2 * NTILE, first_chunk, (WIN - 1) // NTILE + 1)

    def stage(i, _):
        j = jnp.minimum(i, NC - 1)
        spread_keys(jnp.minimum(i - 1, G - 1))
        early_block(i - j, j)

        @pl.when(i < NC - 1)
        def _():
            xcopy(i + 1).wait()
            early_block(1, i, None,
                        [(i + 1, t, [((i + 1) * WIN + k, t) for k in range(WIN)])
                         for t in range(NTILE)], i)
        return 0

    lax.fori_loop(1, NC + 1, stage, 0)
    ecopy().start()

    sv_ref[...] = jnp.dot(pltpu.bitcast(mt_ref[0, V0:LANES // 2, :], BF16), xv_ref[2 * RE],
                          preferred_element_type=F32)
    lax.fori_loop(0, NB - 2, main_block, 0)

    unsafe = jnp.max(jnp.max(flag_ref[...], axis=0))
    ecopy().wait()
    owait(0)
    owait(1)

    @pl.when(unsafe > 0.0)
    def _():
        def block(b, _):
            lo = jnp.where(b < 2, b * RE, 2 * RE + (b - 2) * RM)

            @pl.when(jnp.max(jnp.maximum(flag_ref[b], flag_ref[NB])) > 0.0)
            def _():
                lax.fori_loop(lo, lo + jnp.where(b < 2, RE, RM), true_max_row, 0)
            return 0

        lax.fori_loop(0, NB, block, 0)


@jax.jit
def pallas_standalone__window_attn_twins__vision_kernel(
    x: jax.Array,
    wq: jax.Array,
    wkv: jax.Array,
    wo: jax.Array,
):
    B, H, W, C = x.shape
    nc = H // (WIN * WIN)
    nb = 2 + (H - 2 * RE) // RM
    assert B == 1 and H % (WIN * WIN) == 0 and W % LANES == 0 and W > LANES
    assert (H - 2 * RE) % RM == 0 and nb >= 4 and nc >= max(3, NV // 16) and 2 * RE < WIN * WIN
    assert C % POOL_ROWS == 0 and C % CH_BLK == 0 and (nc * W // LANES) % GROUP == 0
    xt = x.transpose(0, 1, 3, 2).reshape(H, C, W)
    out = pl.pallas_call(
        _kernel,
        in_specs=[pl.BlockSpec(memory_space=pl.ANY)] * 4,
        out_specs=pl.BlockSpec(memory_space=pl.ANY),
        out_shape=jax.ShapeDtypeStruct((H, C, W), x.dtype),
        scratch_shapes=[
            pltpu.VMEM((H, C, W), x.dtype),
            pltpu.VMEM((C, C), wq.dtype),
            pltpu.VMEM((C, 2 * C), wkv.dtype),
            pltpu.VMEM((C, C), wo.dtype),
            pltpu.VMEM((nc, W // 2, C), U32),
            pltpu.VMEM((nc, C // 2, W), U32),
            pltpu.VMEM((C, C), BF16),
            pltpu.VMEM((C, C), BF16),
            pltpu.VMEM((2 * RE, C, W), F32),
            pltpu.VMEM((2 * RE, 8, W), F32),
            pltpu.VMEM((nb + 1, 8, LANES), F32),
            pltpu.VMEM((nc, W, LANES), F32),
            pltpu.VMEM((2 * RE, C, W), x.dtype),
            pltpu.VMEM((2, RM, C, W), x.dtype),
            pltpu.VMEM((C, NV, LANES), F32),
            pltpu.VMEM((NV, W), F32),
            pltpu.VMEM((8, LANES), U32),
            pltpu.SemaphoreType.DMA((3,)),
            pltpu.SemaphoreType.DMA((2 * WIN,)),
            pltpu.SemaphoreType.DMA((nc - 2,)),
            pltpu.SemaphoreType.DMA((3,)),
        ] + [pltpu.VMEM((GROUP * LANES // 2 + 8, W), U32)] * RING
          + [pltpu.VMEM((W // 2 + 8, W), U32)] * RE,
        compiler_params=pltpu.CompilerParams(
            vmem_limit_bytes=100 * 1024 * 1024,
            disable_bounds_checks=True,
            disable_semaphore_checks=True,
        ),
    )(xt, wq, wkv, wo)
    return out.reshape(B, H, C, W).transpose(0, 1, 3, 2)
```

```python
import math

import jax
import jax.numpy as jnp
from jax import lax
import jax.experimental.pallas as pl
import jax.experimental.pallas.tpu as pltpu

F32 = jnp.float32
BF16 = jnp.bfloat16
U32 = jnp.uint32
WIN = 8
LANES = 128
NT = (((1,), (1,)), ((), ()))
TN = (((0,), (0,)), ((), ()))
L_LO, L_HI, V_HI = 1.0, 2.0 ** 30, 2.0 ** 90

RE = 17
RM = 14
NV = 80
LEAD = 2
MIX = 10
SHIFT = 5
SKEW_MAIN = 12
SKEW_A = 2
TIES = 8
GROUP = 2
RING = 7
CH_BLK = 32
POOL_ROWS = 48
OUT_SPLITS = (RM - 2, RM - 1, RM)


def _tree(op, xs):
    xs = list(xs)
    while len(xs) > 1:
        nxt = [op(xs[i], xs[i + 1]) for i in range(0, len(xs) - 1, 2)]
        if len(xs) % 2:
            nxt.append(xs[-1])
        xs = nxt
    return xs[0]


def _red8(reduce, s):
    n, lanes = s.shape[0] // 8, s.shape[1]
    while n > 1:
        r = 2 if n % 2 == 0 else n
        s = reduce(s.reshape(n // r, r, 8, lanes), axis=1)
        n //= r
    return s.reshape(8, lanes)


def _skewed(n, qk, pv, skew, tail=()):
    m = n + skew
    for k in range(m):
        if k < n:
            qk(k)
        if k >= skew:
            pv(k - skew)
        if k >= m - len(tail):
            tail[k - (m - len(tail))]()


def _blk(i, size):
    return pl.ds(i * size if isinstance(i, int) else pl.multiple_of(i * size, size), size)


def _stager(bufs, i):
    spare = bufs[0].shape[0] - 16
    fence = pl.ds(pl.multiple_of((lax.shift_right_logical(i, 20) + 1) * spare, 16), 16)
    zeros = jnp.zeros((16, LANES), BF16)

    def put(k, p):
        bufs[k % len(bufs)][0:p.shape[0], 0:p.shape[1]] = p.astype(BF16)
        bufs[k % len(bufs)][fence, 0:LANES] = zeros

    def get(k, rows, cols):
        return bufs[k % len(bufs)][0:rows, 0:cols]

    return put, get


def _kernel(x_hbm, wq_hbm, wkv_hbm, wo_hbm, o_hbm,
            xv_ref, wq_ref, wkv_ref, wo_ref, mt_ref, vt_ref, a_ref, b_ref,
            acc_ref, l_ref, flag_ref, s_ref, oe_ref, ob_ref, mb_ref, sv_ref, z_ref,
            wsems, xsems0, xsems, osems, *stage_refs):
    H, C, W = xv_ref.shape
    NC = vt_ref.shape[0]
    NTILE = W // LANES
    CR = WIN * WIN
    NB = flag_ref.shape[0] - 1
    V0 = (LANES - NV) // 2
    scale = C ** (-0.5) * math.log2(math.e)
    stage_refs = [r.bitcast(BF16) for r in stage_refs]
    p_refs, pe_refs = stage_refs[:RING], stage_refs[RING:]

    def wcopies():
        pairs = ((wq_hbm, wq_ref), (wkv_hbm, wkv_ref), (wo_hbm, wo_ref))
        return [pltpu.make_async_copy(s, d, wsems.at[i]) for i, (s, d) in enumerate(pairs)]

    def xcopy_first(w):
        rows = pl.ds(w * WIN, WIN)
        return pltpu.make_async_copy(x_hbm.at[rows], xv_ref.at[rows], xsems0.at[w])

    def xcopy(j):
        rows = pl.ds(j * CR, CR)
        return pltpu.make_async_copy(x_hbm.at[rows], xv_ref.at[rows], xsems.at[j - 2])

    def ecopy():
        return pltpu.make_async_copy(oe_ref, o_hbm.at[pl.ds(0, 2 * RE)], osems.at[2])

    def owait(sl):
        pltpu.make_async_copy(ob_ref.at[sl], ob_ref.at[sl], osems.at[sl]).wait()

    def hsum(w, rb, nrows, t):
        hs = None
        for h in range(0, WIN, 2):
            u = (xv_ref[w * WIN + h, rb:rb + nrows, _blk(t, LANES)].astype(F32)
                 + xv_ref[w * WIN + h + 1, rb:rb + nrows, _blk(t, LANES)].astype(F32))
            hs = u if hs is None else hs + u
        return hs

    def fold_lo(a, bit):
        return a + pltpu.roll(a, LANES - bit, 1)

    def merge_hi(a_folded, b, bit):
        lane = lax.broadcasted_iota(jnp.int32, b.shape, 1)
        return jnp.where((lane & bit) == 0, a_folded, b + pltpu.roll(b, bit, 1))

    def project(xst):
        mt = lax.dot_general(xst, a_ref[...], TN, preferred_element_type=F32)
        vt = jnp.dot(b_ref[...], xst, preferred_element_type=F32)
        vbad = _red8(jnp.max, jnp.where(jnp.abs(vt) <= V_HI, 0.0, 1.0))
        return (mt * scale).astype(BF16), vt.astype(BF16), vbad

    def pool(srcs):
        pieces = []
        for rb in range(0, C, POOL_ROWS):
            hs = [hsum(w, rb, POOL_ROWS, t) for w, t in srcs]
            bit = 1
            while len(hs) > 1:
                hs = [merge_hi(fold_lo(hs[k], bit), hs[k + 1], bit) for k in range(0, len(hs), 2)]
                bit *= 2
            pieces.append((hs[0] * (1.0 / CR)).astype(BF16))
        return project(jnp.concatenate(pieces, axis=0))

    def store_keys(j, t, vals):
        mt, vt, vbad = vals
        mt_ref[j, _blk(t, LANES // 2), :] = pltpu.bitcast(mt, U32)
        vt_ref[j, :, _blk(t, LANES)] = pltpu.bitcast(vt, U32)
        flag_ref[NB] = jnp.maximum(flag_ref[NB], vbad)

    def keys_m(j, t=None):
        v = mt_ref[j] if t is None else mt_ref[j, _blk(t, LANES // 2), :]
        return pltpu.bitcast(v, BF16)

    def keys_v(j, t=None):
        v = vt_ref[j] if t is None else vt_ref[j, :, _blk(t, LANES)]
        return pltpu.bitcast(v, BF16)

    def spread_keys(g):
        m = mt_ref[0, pl.ds(pl.multiple_of(V0 + g * 8, 8), 8), :]
        m = pltpu.bitcast(m, BF16).astype(F32)
        for ch in range(C):
            mb_ref[ch, _blk(g, 16), :] = jnp.broadcast_to(m[:, ch:ch + 1], (16, LANES))

    def finish(acc, l):
        lsum = jnp.sum(l, axis=0, keepdims=True)
        bad = jnp.where(jnp.logical_and(lsum >= L_LO, lsum <= L_HI), 0.0, 1.0)
        return ((acc * (1.0 / lsum)).astype(BF16),
                [bad[:, i:i + LANES] for i in range(0, bad.shape[1], LANES)])

    def set_flag(b, bads):
        flag_ref[b] = jnp.broadcast_to(_tree(jnp.maximum, bads), (8, LANES))

    def early_block(half, j, t=None, new_keys=(), i=None):
        r0 = half * RE
        ps, ls, bads, built = {}, {}, [], []
        if new_keys:
            put, get = _stager(pe_refs, i)

        def qk(u):
            p = jnp.exp2(jnp.dot(keys_m(j, t), xv_ref[r0 + u], preferred_element_type=F32))
            if new_keys:
                put(u, p)
            ls[u] = l_ref[r0 + u] + _red8(jnp.sum, p)
            l_ref[r0 + u] = ls[u]
            ps[u] = p

        def pv(u):
            p = ps.pop(u)
            p = get(u, *p.shape) if new_keys else p.astype(BF16)
            acc = acc_ref[r0 + u] + jnp.dot(keys_v(j, t), p, preferred_element_type=F32)
            acc_ref[r0 + u] = acc
            if not new_keys:
                oe_ref[r0 + u], bad = finish(acc, ls[u])
                bads.extend(bad)

        _skewed(RE, qk, pv, RE if new_keys else SKEW_A,
                [lambda srcs=srcs: built.append(pool(srcs)) for _, _, srcs in new_keys])
        for (jn, tn, _), vals in zip(new_keys, built):
            store_keys(jn, tn, vals)
        if bads:
            set_flag(half, bads)

    def main_block(b, _):
        slot = lax.rem(b, 2)
        row0 = 2 * RE + b * RM

        @pl.when(b >= 2)
        def _():
            owait(slot)

        put, get = _stager(p_refs, b)
        order = list(range(1, NC * NTILE))
        order.insert(len(order) - MIX, 0)
        items = [(u, t, kt) for u in range(RM) for t in range(NTILE) for kt in order]
        per, end = len(order) * TIES, len(items) * TIES
        work = {}
        for q in range(LEAD, RM * NTILE + LEAD):
            for ch in range(C):
                pos = (q - LEAD) * per + (2 * ch + 1) * per // (2 * C) + SHIFT
                work.setdefault(min(pos, end), []).append((q, ch))
        never = jnp.broadcast_to((z_ref[:, :C] != 0)[None], (TIES, 8, C))
        sv, ops, qops, vops, st, pend, bads, last = {}, {}, {}, {}, {}, [], [], [0, None]

        def vpu(n):
            for q, ch in work.get(n, ()):
                key, chs = (q, ch // CH_BLK), _blk(ch // CH_BLK, CH_BLK)
                if key not in ops:
                    u, t = q // NTILE, q % NTILE
                    row = row0 + u if u < RM else jnp.minimum(row0 + u, H - 1)
                    ops[key] = (xv_ref[row, chs, _blk(t, LANES)].astype(F32)[None], mb_ref[chs])
                xb, mb = ops[key]
                c = ch % CH_BLK
                term = mb[c:c + 1] * xb[:, c:c + 1, :]
                sv[q] = term if ch == 0 else sv[q] + term
            if n in work:
                last[0] = (last[0] + 1) % (NV // 8)
                last[1] = sv[q][:, last[0] * 8:last[0] * 8 + 8, :C]
            return last[1]

        def qk(k):
            u, t, kt = items[k]
            if (u, t) not in qops:
                qops[(u, t)] = (xv_ref[row0 + u, :, _blk(t, LANES)], mt_ref[...])
            xt, mt = qops[(u, t)]
            rows = (LANES - NV if kt == 0 else LANES) // 2
            j, lo = kt // NTILE, (kt % NTILE) * (LANES // 2)
            tie = [vpu(k * TIES + a) for a in range(TIES)][TIES - rows // 8:]
            mt = mt[j:j + 1, lo:lo + rows].reshape(rows // 8, 8, C)
            if tie[0] is not None:
                tie = pltpu.bitcast(jnp.concatenate(tie, axis=0), U32)
                mt = lax.select(never[:rows // 8], tie, mt)
            s = jnp.dot(pltpu.bitcast(mt.reshape(rows, C), BF16), xt, preferred_element_type=F32)
            pend.append(s)
            if kt == 0:
                q = u * NTILE + t
                pend.append(sv_ref[:, _blk(t, LANES)] if q < LEAD else sv[q][0])
            if k % GROUP == GROUP - 1:
                p = jnp.exp2(jnp.concatenate(pend, axis=0))
                del pend[:]
                put(k // GROUP, p)
                lc = _red8(jnp.sum, p)
                acc, l = st.get((u, t), (None, None))
                st[(u, t)] = (acc, lc if l is None else l + lc)

        def pv(k):
            u, t, kt = items[k]
            if (u, t) not in vops:
                vops[(u, t)] = pltpu.bitcast(vt_ref[...], BF16)
            if k % GROUP == 0:
                vops["p"] = get(k // GROUP, GROUP * LANES, LANES)
            vt = vops[(u, t)][kt // NTILE, :, (kt % NTILE) * LANES:(kt % NTILE + 1) * LANES]
            p = vops["p"][(k % GROUP) * LANES:(k % GROUP + 1) * LANES]
            y = jnp.dot(vt, p, preferred_element_type=F32)
            acc, l = st[(u, t)]
            acc = y if acc is None else acc + y
            st[(u, t)] = (acc, l)
            if kt == order[-1]:
                ob_ref[slot, u, :, _blk(t, LANES)], bad = finish(acc, l)
                bads.extend(bad)
                if t == NTILE - 1 and u + 1 in OUT_SPLITS:
                    lo = max([0] + [e for e in OUT_SPLITS if e < u + 1])
                    pltpu.make_async_copy(ob_ref.at[slot, pl.ds(lo, u + 1 - lo)],
                                          o_hbm.at[pl.ds(row0 + lo, u + 1 - lo)],
                                          osems.at[slot]).start()

        _skewed(len(items), qk, pv, SKEW_MAIN)
        vpu(end)
        for t in range(LEAD):
            sv_ref[:, _blk(t, LANES)] = sv[RM * NTILE + t][0]
        set_flag(2 + b, bads)
        return 0

    def true_max_row(r, _):
        def tile(t, _):
            lanes = _blk(t, LANES)

            def qk(c, m):
                s = jnp.dot(keys_m(c), xv_ref[r, :, lanes], preferred_element_type=F32)
                s_ref[c] = s
                return jnp.maximum(m, _red8(jnp.max, s))

            m = lax.fori_loop(0, NC, qk, jnp.full((8, LANES), -jnp.inf, F32))
            m = jnp.max(m, axis=0, keepdims=True)

            def pv(c, carry):
                acc, l = carry
                p = jnp.exp2(s_ref[c] - m)
                return (acc + jnp.dot(keys_v(c), p.astype(BF16), preferred_element_type=F32),
                        l + _red8(jnp.sum, p))

            acc, l = lax.fori_loop(0, NC, pv,
                                   (jnp.zeros((C, LANES), F32), jnp.zeros((8, LANES), F32)))
            oe_ref[0, :, lanes] = (acc / jnp.sum(l, axis=0, keepdims=True)).astype(BF16)
            return 0

        lax.fori_loop(0, NTILE, tile, 0)
        cp = pltpu.make_async_copy(oe_ref.at[0], o_hbm.at[r], osems.at[2])
        cp.start()
        cp.wait()
        return 0

    for cp in wcopies():
        cp.start()
    for w in range(2 * WIN):
        xcopy_first(w).start(priority=1)
    for j in range(2, NC):
        xcopy(j).start(priority=1)
    flag_ref[...] = jnp.zeros(flag_ref.shape, F32)
    z_ref[...] = jnp.zeros(z_ref.shape, U32)

    def zero(r, _):
        acc_ref[r] = jnp.zeros((C, W), F32)
        l_ref[r] = jnp.zeros((8, W), F32)
        return 0

    lax.fori_loop(0, 2 * RE, zero, 0)
    for cp in wcopies():
        cp.wait()
    wkv = wkv_ref[...]
    a_ref[...] = lax.dot_general(wkv[:, :C], wq_ref[...], NT, preferred_element_type=F32).astype(BF16)
    b_ref[...] = jnp.dot(wkv[:, C:], wo_ref[...], preferred_element_type=F32).T.astype(BF16)

    stack = []
    for q in range(WIN):
        if q % NTILE == 0:
            xcopy_first(q // NTILE).wait()
        cur = hsum(q // NTILE, 0, C, q % NTILE)
        bit = 1
        while q & bit:
            cur = merge_hi(stack.pop(), cur, bit)
            bit *= 2
        stack.append(fold_lo(cur, bit) if q < WIN - 1 else cur)
    store_keys(0, 0, project((stack[0] * (1.0 / CR)).astype(BF16)))

    def first_chunk(n, done):
        half = lax.rem(n, 2)
        last = jnp.maximum(lax.div(WIN * n + WIN - 1, NTILE),
                           lax.div((half + 1) * RE - 1, WIN))
        need = jnp.maximum(done, last + 1)

        def wait_row(w, _):
            xcopy_first(w).wait()
            return 0

        lax.fori_loop(done, need, wait_row, 0)
        srcs = [(lax.div(WIN * n + i, NTILE), lax.rem(WIN * n + i, NTILE)) for i in range(WIN)]
        early_block(half, 0, lax.div(n, 2), [(lax.div(n, NTILE), lax.rem(n, NTILE), srcs)], n)
        return need

    lax.fori_loop(0, 2 * NTILE, first_chunk, (WIN - 1) // NTILE + 1)

    def stage(i, _):
        j = jnp.minimum(i, NC - 1)
        spread_keys(jnp.minimum(i - 1, NV // 16 - 1))
        early_block(i - j, j)

        @pl.when(i < NC - 1)
        def _():
            xcopy(i + 1).wait()
            early_block(1, i, None,
                        [(i + 1, t, [((i + 1) * WIN + k, t) for k in range(WIN)])
                         for t in range(NTILE)], i)
        return 0

    lax.fori_loop(1, NC + 1, stage, 0)
    ecopy().start()

    sv_ref[...] = jnp.dot(pltpu.bitcast(mt_ref[0, V0:LANES // 2, :], BF16),
                          xv_ref[2 * RE, :, 0:LEAD * LANES], preferred_element_type=F32)
    lax.fori_loop(0, NB - 2, main_block, 0)

    unsafe = jnp.max(jnp.max(flag_ref[...], axis=0))
    ecopy().wait()
    owait(0)
    owait(1)

    @pl.when(unsafe > 0.0)
    def _():
        def block(b, _):
            lo = jnp.where(b < 2, b * RE, 2 * RE + (b - 2) * RM)

            @pl.when(jnp.max(jnp.maximum(flag_ref[b], flag_ref[NB])) > 0.0)
            def _():
                lax.fori_loop(lo, lo + jnp.where(b < 2, RE, RM), true_max_row, 0)
            return 0

        lax.fori_loop(0, NB, block, 0)


@jax.jit
def pallas_standalone__window_attn_twins__vision_kernel(
    x: jax.Array,
    wq: jax.Array,
    wkv: jax.Array,
    wo: jax.Array,
):
    B, H, W, C = x.shape
    nc = H // (WIN * WIN)
    nb = 2 + (H - 2 * RE) // RM
    assert B == 1 and H % (WIN * WIN) == 0 and W % LANES == 0 and W > LANES
    assert (H - 2 * RE) % RM == 0 and nb >= 4 and nc >= max(3, NV // 16) and 2 * RE < WIN * WIN
    assert C % POOL_ROWS == 0 and C % CH_BLK == 0 and (nc * W // LANES) % GROUP == 0
    assert TIES * 16 == LANES and 2 <= LEAD <= W // LANES and SHIFT <= TIES and MIX < nc * W // LANES
    xt = x.transpose(0, 1, 3, 2).reshape(H, C, W)
    out = pl.pallas_call(
        _kernel,
        in_specs=[pl.BlockSpec(memory_space=pl.ANY)] * 4,
        out_specs=pl.BlockSpec(memory_space=pl.ANY),
        out_shape=jax.ShapeDtypeStruct((H, C, W), x.dtype),
        scratch_shapes=[
            pltpu.VMEM((H, C, W), x.dtype),
            pltpu.VMEM((C, C), wq.dtype),
            pltpu.VMEM((C, 2 * C), wkv.dtype),
            pltpu.VMEM((C, C), wo.dtype),
            pltpu.VMEM((nc, W // 2, C), U32),
            pltpu.VMEM((nc, C // 2, W), U32),
            pltpu.VMEM((C, C), BF16),
            pltpu.VMEM((C, C), BF16),
            pltpu.VMEM((2 * RE, C, W), F32),
            pltpu.VMEM((2 * RE, 8, W), F32),
            pltpu.VMEM((nb + 1, 8, LANES), F32),
            pltpu.VMEM((nc, W, LANES), F32),
            pltpu.VMEM((2 * RE, C, W), x.dtype),
            pltpu.VMEM((2, RM, C, W), x.dtype),
            pltpu.VMEM((C, NV, LANES), F32),
            pltpu.VMEM((NV, LEAD * LANES), F32),
            pltpu.VMEM((8, LANES), U32),
            pltpu.SemaphoreType.DMA((3,)),
            pltpu.SemaphoreType.DMA((2 * WIN,)),
            pltpu.SemaphoreType.DMA((nc - 2,)),
            pltpu.SemaphoreType.DMA((3,)),
        ] + [pltpu.VMEM((GROUP * LANES // 2 + 8, W), U32)] * RING
          + [pltpu.VMEM((W // 2 + 8, W), U32)] * RE,
        compiler_params=pltpu.CompilerParams(
            vmem_limit_bytes=100 * 1024 * 1024,
            disable_bounds_checks=True,
            disable_semaphore_checks=True,
        ),
    )(xt, wq, wkv, wo)
    return out.reshape(B, H, C, W).transpose(0, 1, 3, 2)
```

```python
import math

import jax
import jax.numpy as jnp
from jax import lax
import jax.experimental.pallas as pl
import jax.experimental.pallas.tpu as pltpu

F32 = jnp.float32
BF16 = jnp.bfloat16
U32 = jnp.uint32
WIN = 8
LANES = 128
NT = (((1,), (1,)), ((), ()))
TN = (((0,), (0,)), ((), ()))
L_LO, L_HI, V_HI = 1.0, 2.0 ** 30, 2.0 ** 90

RE = 17
RM = 14
NV = 80
LEAD = 2
MIX = 10
SHIFT = 5
SKEW_MAIN = 12
SKEW_A = 2
TIES = 8
GROUP = 3
RING = 10
CH_BLK = 96
POOL_ROWS = 48
OUT_SPLITS = (RM - 2, RM - 1, RM)


def _tree(op, xs):
    xs = list(xs)
    while len(xs) > 1:
        nxt = [op(xs[i], xs[i + 1]) for i in range(0, len(xs) - 1, 2)]
        if len(xs) % 2:
            nxt.append(xs[-1])
        xs = nxt
    return xs[0]


def _red8(reduce, s):
    n, lanes = s.shape[0] // 8, s.shape[1]
    while n > 1:
        r = 2 if n % 2 == 0 else n
        s = reduce(s.reshape(n // r, r, 8, lanes), axis=1)
        n //= r
    return s.reshape(8, lanes)


def _skewed(n, qk, pv, skew, tail=()):
    m = n + skew
    for k in range(m):
        if k < n:
            qk(k)
        if k >= skew:
            pv(k - skew)
        if k >= m - len(tail):
            tail[k - (m - len(tail))]()


def _blk(i, size):
    return pl.ds(i * size if isinstance(i, int) else pl.multiple_of(i * size, size), size)


def _stager(bufs, i):
    spare = bufs[0].shape[0] - 16
    fence = pl.ds(pl.multiple_of((lax.shift_right_logical(i, 20) + 1) * spare, 16), 16)
    zeros = jnp.zeros((16, LANES), BF16)

    def put(k, p):
        bufs[k % len(bufs)][0:p.shape[0], 0:p.shape[1]] = p.astype(BF16)
        bufs[k % len(bufs)][fence, 0:LANES] = zeros

    def get(k, rows, cols):
        return bufs[k % len(bufs)][0:rows, 0:cols]

    return put, get


def _kernel(x_hbm, wq_hbm, wkv_hbm, wo_hbm, o_hbm,
            xv_ref, wq_ref, wkv_ref, wo_ref, mt_ref, vt_ref, a_ref, b_ref,
            acc_ref, l_ref, flag_ref, s_ref, oe_ref, ob_ref, mb_ref, sv_ref, z_ref,
            wsems, xsems0, xsems, osems, *stage_refs):
    H, C, W = xv_ref.shape
    NC = vt_ref.shape[0]
    NTILE = W // LANES
    CR = WIN * WIN
    NB = flag_ref.shape[0] - 1
    V0 = (LANES - NV) // 2
    scale = C ** (-0.5) * math.log2(math.e)
    stage_refs = [r.bitcast(BF16) for r in stage_refs]
    p_refs, pe_refs = stage_refs[:RING], stage_refs[RING:]

    def wcopies():
        pairs = ((wq_hbm, wq_ref), (wkv_hbm, wkv_ref), (wo_hbm, wo_ref))
        return [pltpu.make_async_copy(s, d, wsems.at[i]) for i, (s, d) in enumerate(pairs)]

    def xcopy_first(w):
        rows = pl.ds(w * WIN, WIN)
        return pltpu.make_async_copy(x_hbm.at[rows], xv_ref.at[rows], xsems0.at[w])

    def xcopy(j):
        rows = pl.ds(j * CR, CR)
        return pltpu.make_async_copy(x_hbm.at[rows], xv_ref.at[rows], xsems.at[j - 2])

    def ecopy():
        return pltpu.make_async_copy(oe_ref, o_hbm.at[pl.ds(0, 2 * RE)], osems.at[2])

    def owait(sl):
        pltpu.make_async_copy(ob_ref.at[sl], ob_ref.at[sl], osems.at[sl]).wait()

    def hsum(w, rb, nrows, t):
        hs = None
        for h in range(0, WIN, 2):
            u = (xv_ref[w * WIN + h, rb:rb + nrows, _blk(t, LANES)].astype(F32)
                 + xv_ref[w * WIN + h + 1, rb:rb + nrows, _blk(t, LANES)].astype(F32))
            hs = u if hs is None else hs + u
        return hs

    def fold_lo(a, bit):
        return a + pltpu.roll(a, LANES - bit, 1)

    def merge_hi(a_folded, b, bit):
        lane = lax.broadcasted_iota(jnp.int32, b.shape, 1)
        return jnp.where((lane & bit) == 0, a_folded, b + pltpu.roll(b, bit, 1))

    def project(xst):
        mt = lax.dot_general(xst, a_ref[...], TN, preferred_element_type=F32)
        vt = jnp.dot(b_ref[...], xst, preferred_element_type=F32)
        vbad = _red8(jnp.max, jnp.where(jnp.abs(vt) <= V_HI, 0.0, 1.0))
        return (mt * scale).astype(BF16), vt.astype(BF16), vbad

    def pool(srcs):
        pieces = []
        for rb in range(0, C, POOL_ROWS):
            hs = [hsum(w, rb, POOL_ROWS, t) for w, t in srcs]
            bit = 1
            while len(hs) > 1:
                hs = [merge_hi(fold_lo(hs[k], bit), hs[k + 1], bit) for k in range(0, len(hs), 2)]
                bit *= 2
            pieces.append((hs[0] * (1.0 / CR)).astype(BF16))
        return project(jnp.concatenate(pieces, axis=0))

    def store_keys(j, t, vals):
        mt, vt, vbad = vals
        mt_ref[j, _blk(t, LANES // 2), :] = pltpu.bitcast(mt, U32)
        vt_ref[j, :, _blk(t, LANES)] = pltpu.bitcast(vt, U32)
        flag_ref[NB] = jnp.maximum(flag_ref[NB], vbad)

    def keys_m(j, t=None):
        v = mt_ref[j] if t is None else mt_ref[j, _blk(t, LANES // 2), :]
        return pltpu.bitcast(v, BF16)

    def keys_v(j, t=None):
        v = vt_ref[j] if t is None else vt_ref[j, :, _blk(t, LANES)]
        return pltpu.bitcast(v, BF16)

    def spread_keys(g):
        m = mt_ref[0, pl.ds(pl.multiple_of(V0 + g * 8, 8), 8), :]
        m = pltpu.bitcast(m, BF16).astype(F32)
        for ch in range(C):
            mb_ref[ch, _blk(g, 16), :] = jnp.broadcast_to(m[:, ch:ch + 1], (16, LANES))

    def finish(acc, l):
        lsum = jnp.sum(l, axis=0, keepdims=True)
        bad = jnp.where(jnp.logical_and(lsum >= L_LO, lsum <= L_HI), 0.0, 1.0)
        return ((acc * (1.0 / lsum)).astype(BF16),
                [bad[:, i:i + LANES] for i in range(0, bad.shape[1], LANES)])

    def set_flag(b, bads):
        flag_ref[b] = jnp.broadcast_to(_tree(jnp.maximum, bads), (8, LANES))

    def early_block(half, j, t=None, new_keys=(), i=None):
        r0 = half * RE
        ps, ls, bads, built = {}, {}, [], []
        if new_keys:
            put, get = _stager(pe_refs, i)

        def qk(u):
            p = jnp.exp2(jnp.dot(keys_m(j, t), xv_ref[r0 + u], preferred_element_type=F32))
            if new_keys:
                put(u, p)
            ls[u] = l_ref[r0 + u] + _red8(jnp.sum, p)
            l_ref[r0 + u] = ls[u]
            ps[u] = p

        def pv(u):
            p = ps.pop(u)
            p = get(u, *p.shape) if new_keys else p.astype(BF16)
            acc = acc_ref[r0 + u] + jnp.dot(keys_v(j, t), p, preferred_element_type=F32)
            acc_ref[r0 + u] = acc
            if not new_keys:
                oe_ref[r0 + u], bad = finish(acc, ls[u])
                bads.extend(bad)

        _skewed(RE, qk, pv, RE if new_keys else SKEW_A,
                [lambda srcs=srcs: built.append(pool(srcs)) for _, _, srcs in new_keys])
        for (jn, tn, _), vals in zip(new_keys, built):
            store_keys(jn, tn, vals)
        if bads:
            set_flag(half, bads)

    def main_block(b, _):
        slot = lax.rem(b, 2)
        row0 = 2 * RE + b * RM

        @pl.when(b >= 2)
        def _():
            owait(slot)

        put, get = _stager(p_refs, b)
        order = list(range(1, NC * NTILE))
        order.insert(len(order) - MIX, 0)
        items = [(u, t, kt) for u in range(RM) for t in range(NTILE) for kt in order]
        per, end = len(order) * TIES, len(items) * TIES
        work = {}
        for q in range(LEAD, RM * NTILE + LEAD):
            for ch in range(C):
                pos = (q - LEAD) * per + (2 * ch + 1) * per // (2 * C) + SHIFT
                work.setdefault(min(pos, end), []).append((q, ch))
        never = jnp.broadcast_to((z_ref[:, :C] != 0)[None], (TIES, 8, C))
        sv, ops, qops, vops, st, pend, bads, last = {}, {}, {}, {}, {}, [], [], [0, None]

        def vpu(n):
            for q, ch in work.get(n, ()):
                key, chs = (q, ch // CH_BLK), _blk(ch // CH_BLK, CH_BLK)
                if key not in ops:
                    u, t = q // NTILE, q % NTILE
                    row = row0 + u if u < RM else jnp.minimum(row0 + u, H - 1)
                    ops[key] = (xv_ref[row, chs, _blk(t, LANES)].astype(F32)[None], mb_ref[chs])
                xb, mb = ops[key]
                c = ch % CH_BLK
                term = mb[c:c + 1] * xb[:, c:c + 1, :]
                sv[q] = term if ch == 0 else sv[q] + term
            if n in work:
                last[0] = (last[0] + 1) % (NV // 8)
                last[1] = sv[q][:, last[0] * 8:last[0] * 8 + 8, :C]
            return last[1]

        def qk(k):
            u, t, kt = items[k]
            if (u, t) not in qops:
                qops[(u, t)] = (xv_ref[row0 + u, :, _blk(t, LANES)], mt_ref[...])
            xt, mt = qops[(u, t)]
            rows = (LANES - NV if kt == 0 else LANES) // 2
            j, lo = kt // NTILE, (kt % NTILE) * (LANES // 2)
            tie = [vpu(k * TIES + a) for a in range(TIES)][TIES - rows // 8:]
            mt = mt[j:j + 1, lo:lo + rows].reshape(rows // 8, 8, C)
            if tie[0] is not None:
                tie = pltpu.bitcast(jnp.concatenate(tie, axis=0), U32)
                mt = lax.select(never[:rows // 8], tie, mt)
            s = jnp.dot(pltpu.bitcast(mt.reshape(rows, C), BF16), xt, preferred_element_type=F32)
            pend.append(s)
            if kt == 0:
                q = u * NTILE + t
                pend.append(sv_ref[:, _blk(t, LANES)] if q < LEAD else sv[q][0])
            if k % GROUP == GROUP - 1:
                p = jnp.exp2(jnp.concatenate(pend, axis=0))
                del pend[:]
                put(k // GROUP, p)
                lc = _red8(jnp.sum, p)
                acc, l = st.get((u, t), (None, None))
                st[(u, t)] = (acc, lc if l is None else l + lc)

        def pv(k):
            u, t, kt = items[k]
            if (u, t) not in vops:
                vops[(u, t)] = pltpu.bitcast(vt_ref[...], BF16)
            if k % GROUP == 0:
                vops["p"] = get(k // GROUP, GROUP * LANES, LANES)
            vt = vops[(u, t)][kt // NTILE, :, (kt % NTILE) * LANES:(kt % NTILE + 1) * LANES]
            p = vops["p"][(k % GROUP) * LANES:(k % GROUP + 1) * LANES]
            y = jnp.dot(vt, p, preferred_element_type=F32)
            acc, l = st[(u, t)]
            acc = y if acc is None else acc + y
            st[(u, t)] = (acc, l)
            if kt == order[-1]:
                ob_ref[slot, u, :, _blk(t, LANES)], bad = finish(acc, l)
                bads.extend(bad)
                if t == NTILE - 1 and u + 1 in OUT_SPLITS:
                    lo = max([0] + [e for e in OUT_SPLITS if e < u + 1])
                    pltpu.make_async_copy(ob_ref.at[slot, pl.ds(lo, u + 1 - lo)],
                                          o_hbm.at[pl.ds(row0 + lo, u + 1 - lo)],
                                          osems.at[slot]).start()

        _skewed(len(items), qk, pv, SKEW_MAIN)
        vpu(end)
        for t in range(LEAD):
            sv_ref[:, _blk(t, LANES)] = sv[RM * NTILE + t][0]
        set_flag(2 + b, bads)
        return 0

    def true_max_row(r, _):
        def tile(t, _):
            lanes = _blk(t, LANES)

            def qk(c, m):
                s = jnp.dot(keys_m(c), xv_ref[r, :, lanes], preferred_element_type=F32)
                s_ref[c] = s
                return jnp.maximum(m, _red8(jnp.max, s))

            m = lax.fori_loop(0, NC, qk, jnp.full((8, LANES), -jnp.inf, F32))
            m = jnp.max(m, axis=0, keepdims=True)

            def pv(c, carry):
                acc, l = carry
                p = jnp.exp2(s_ref[c] - m)
                return (acc + jnp.dot(keys_v(c), p.astype(BF16), preferred_element_type=F32),
                        l + _red8(jnp.sum, p))

            acc, l = lax.fori_loop(0, NC, pv,
                                   (jnp.zeros((C, LANES), F32), jnp.zeros((8, LANES), F32)))
            oe_ref[0, :, lanes] = (acc / jnp.sum(l, axis=0, keepdims=True)).astype(BF16)
            return 0

        lax.fori_loop(0, NTILE, tile, 0)
        cp = pltpu.make_async_copy(oe_ref.at[0], o_hbm.at[r], osems.at[2])
        cp.start()
        cp.wait()
        return 0

    for cp in wcopies():
        cp.start()
    for w in range(2 * WIN):
        xcopy_first(w).start(priority=1)
    for j in range(2, NC):
        xcopy(j).start(priority=1)
    flag_ref[...] = jnp.zeros(flag_ref.shape, F32)
    z_ref[...] = jnp.zeros(z_ref.shape, U32)

    def zero(r, _):
        acc_ref[r] = jnp.zeros((C, W), F32)
        l_ref[r] = jnp.zeros((8, W), F32)
        return 0

    lax.fori_loop(0, 2 * RE, zero, 0)
    for cp in wcopies():
        cp.wait()
    wkv = wkv_ref[...]
    a_ref[...] = lax.dot_general(wkv[:, :C], wq_ref[...], NT, preferred_element_type=F32).astype(BF16)
    b_ref[...] = jnp.dot(wkv[:, C:], wo_ref[...], preferred_element_type=F32).T.astype(BF16)

    stack = []
    for q in range(WIN):
        if q % NTILE == 0:
            xcopy_first(q // NTILE).wait()
        cur = hsum(q // NTILE, 0, C, q % NTILE)
        bit = 1
        while q & bit:
            cur = merge_hi(stack.pop(), cur, bit)
            bit *= 2
        stack.append(fold_lo(cur, bit) if q < WIN - 1 else cur)
    store_keys(0, 0, project((stack[0] * (1.0 / CR)).astype(BF16)))

    def first_chunk(n, done):
        half = lax.rem(n, 2)
        last = jnp.maximum(lax.div(WIN * n + WIN - 1, NTILE),
                           lax.div((half + 1) * RE - 1, WIN))
        need = jnp.maximum(done, last + 1)

        def wait_row(w, _):
            xcopy_first(w).wait()
            return 0

        lax.fori_loop(done, need, wait_row, 0)
        srcs = [(lax.div(WIN * n + i, NTILE), lax.rem(WIN * n + i, NTILE)) for i in range(WIN)]
        early_block(half, 0, lax.div(n, 2), [(lax.div(n, NTILE), lax.rem(n, NTILE), srcs)], n)
        return need

    lax.fori_loop(0, 2 * NTILE, first_chunk, (WIN - 1) // NTILE + 1)

    def stage(i, _):
        j = jnp.minimum(i, NC - 1)
        spread_keys(jnp.minimum(i - 1, NV // 16 - 1))
        early_block(i - j, j)

        @pl.when(i < NC - 1)
        def _():
            xcopy(i + 1).wait()
            early_block(1, i, None,
                        [(i + 1, t, [((i + 1) * WIN + k, t) for k in range(WIN)])
                         for t in range(NTILE)], i)
        return 0

    lax.fori_loop(1, NC + 1, stage, 0)
    ecopy().start()

    sv_ref[...] = jnp.dot(pltpu.bitcast(mt_ref[0, V0:LANES // 2, :], BF16),
                          xv_ref[2 * RE, :, 0:LEAD * LANES], preferred_element_type=F32)
    lax.fori_loop(0, NB - 2, main_block, 0)

    unsafe = jnp.max(jnp.max(flag_ref[...], axis=0))
    ecopy().wait()
    owait(0)
    owait(1)

    @pl.when(unsafe > 0.0)
    def _():
        def block(b, _):
            lo = jnp.where(b < 2, b * RE, 2 * RE + (b - 2) * RM)

            @pl.when(jnp.max(jnp.maximum(flag_ref[b], flag_ref[NB])) > 0.0)
            def _():
                lax.fori_loop(lo, lo + jnp.where(b < 2, RE, RM), true_max_row, 0)
            return 0

        lax.fori_loop(0, NB, block, 0)


@jax.jit
def pallas_standalone__window_attn_twins__vision_kernel(
    x: jax.Array,
    wq: jax.Array,
    wkv: jax.Array,
    wo: jax.Array,
):
    B, H, W, C = x.shape
    nc = H // (WIN * WIN)
    nb = 2 + (H - 2 * RE) // RM
    assert B == 1 and H % (WIN * WIN) == 0 and W % LANES == 0 and W > LANES
    assert (H - 2 * RE) % RM == 0 and nb >= 4 and nc >= max(3, NV // 16) and 2 * RE < WIN * WIN
    assert C % POOL_ROWS == 0 and C % CH_BLK == 0 and (nc * W // LANES) % GROUP == 0
    assert TIES * 16 == LANES and 2 <= LEAD <= W // LANES and SHIFT <= TIES and MIX < nc * W // LANES
    assert GROUP <= SKEW_MAIN < RING * GROUP + GROUP - 1
    xt = x.transpose(0, 1, 3, 2).reshape(H, C, W)
    out = pl.pallas_call(
        _kernel,
        in_specs=[pl.BlockSpec(memory_space=pl.ANY)] * 4,
        out_specs=pl.BlockSpec(memory_space=pl.ANY),
        out_shape=jax.ShapeDtypeStruct((H, C, W), x.dtype),
        scratch_shapes=[
            pltpu.VMEM((H, C, W), x.dtype),
            pltpu.VMEM((C, C), wq.dtype),
            pltpu.VMEM((C, 2 * C), wkv.dtype),
            pltpu.VMEM((C, C), wo.dtype),
            pltpu.VMEM((nc, W // 2, C), U32),
            pltpu.VMEM((nc, C // 2, W), U32),
            pltpu.VMEM((C, C), BF16),
            pltpu.VMEM((C, C), BF16),
            pltpu.VMEM((2 * RE, C, W), F32),
            pltpu.VMEM((2 * RE, 8, W), F32),
            pltpu.VMEM((nb + 1, 8, LANES), F32),
            pltpu.VMEM((nc, W, LANES), F32),
            pltpu.VMEM((2 * RE, C, W), x.dtype),
            pltpu.VMEM((2, RM, C, W), x.dtype),
            pltpu.VMEM((C, NV, LANES), F32),
            pltpu.VMEM((NV, LEAD * LANES), F32),
            pltpu.VMEM((8, LANES), U32),
            pltpu.SemaphoreType.DMA((3,)),
            pltpu.SemaphoreType.DMA((2 * WIN,)),
            pltpu.SemaphoreType.DMA((nc - 2,)),
            pltpu.SemaphoreType.DMA((3,)),
        ] + [pltpu.VMEM((GROUP * LANES // 2 + 8, W), U32)] * RING
          + [pltpu.VMEM((W // 2 + 8, W), U32)] * RE,
        compiler_params=pltpu.CompilerParams(
            vmem_limit_bytes=100 * 1024 * 1024,
            disable_bounds_checks=True,
            disable_semaphore_checks=True,
        ),
    )(xt, wq, wkv, wo)
    return out.reshape(B, H, C, W).transpose(0, 1, 3, 2)
```

```python
import math

import jax
import jax.numpy as jnp
from jax import lax
import jax.experimental.pallas as pl
import jax.experimental.pallas.tpu as pltpu

F32 = jnp.float32
BF16 = jnp.bfloat16
U32 = jnp.uint32
WIN = 8
LANES = 128
NT = (((1,), (1,)), ((), ()))
TN = (((0,), (0,)), ((), ()))
L_LO, L_HI, V_HI = 1.0, 2.0 ** 30, 2.0 ** 90

RE = 17
RM = 14
NV = 64
LEAD = 2
MIX = 10
SHIFT = 2
SKEW_MAIN = 12
SKEW_A = 2
TIES = 4
GROUP = 2
RING = 9
POOL_ROWS = 48
OUT_SPLITS = (RM - 2, RM - 1, RM)


def _tree(op, xs):
    xs = list(xs)
    while len(xs) > 1:
        nxt = [op(xs[i], xs[i + 1]) for i in range(0, len(xs) - 1, 2)]
        if len(xs) % 2:
            nxt.append(xs[-1])
        xs = nxt
    return xs[0]


def _red8(reduce, s):
    n, lanes = s.shape[0] // 8, s.shape[1]
    while n > 1:
        r = 2 if n % 2 == 0 else n
        s = reduce(s.reshape(n // r, r, 8, lanes), axis=1)
        n //= r
    return s.reshape(8, lanes)


def _skewed(n, qk, pv, skew, tail=()):
    m = n + skew
    for k in range(m):
        if k < n:
            qk(k)
        if k >= skew:
            pv(k - skew)
        if k >= m - len(tail):
            tail[k - (m - len(tail))]()


def _blk(i, size):
    return pl.ds(i * size if isinstance(i, int) else pl.multiple_of(i * size, size), size)


def _regroup(p):
    n, cols = p.shape
    p = p.reshape(n // LANES, LANES // 16, 16, cols)
    return jnp.concatenate([p[:, :, :8], p[:, :, 8:]], axis=1).reshape(n, cols)


def _kernel(x_hbm, wq_hbm, wkv_hbm, wo_hbm, o_hbm,
            xv_ref, wq_ref, wkv_ref, wo_ref, mt_ref, vt_ref, a_ref, b_ref,
            acc_ref, l_ref, flag_ref, s_ref, oe_ref, ob_ref, mb_ref, sv_ref, z_ref,
            wsems, xsems0, xsems, osems, *p_refs):
    H, C, W = xv_ref.shape
    NC = vt_ref.shape[0]
    NTILE = W // LANES
    CR = WIN * WIN
    NB = flag_ref.shape[0] - 1
    V0 = (LANES - NV) // 2
    scale = C ** (-0.5) * math.log2(math.e)

    def wcopies():
        pairs = ((wq_hbm, wq_ref), (wkv_hbm, wkv_ref), (wo_hbm, wo_ref))
        return [pltpu.make_async_copy(s, d, wsems.at[i]) for i, (s, d) in enumerate(pairs)]

    def xcopy_first(w):
        rows = pl.ds(w * WIN, WIN)
        return pltpu.make_async_copy(x_hbm.at[rows], xv_ref.at[rows], xsems0.at[w])

    def xcopy(j):
        rows = pl.ds(j * CR, CR)
        return pltpu.make_async_copy(x_hbm.at[rows], xv_ref.at[rows], xsems.at[j - 2])

    def ecopy():
        return pltpu.make_async_copy(oe_ref, o_hbm.at[pl.ds(0, 2 * RE)], osems.at[2])

    def owait(sl):
        pltpu.make_async_copy(ob_ref.at[sl], ob_ref.at[sl], osems.at[sl]).wait()

    def hsum(w, rb, nrows, t):
        hs = None
        for h in range(0, WIN, 2):
            u = (xv_ref[w * WIN + h, rb:rb + nrows, _blk(t, LANES)].astype(F32)
                 + xv_ref[w * WIN + h + 1, rb:rb + nrows, _blk(t, LANES)].astype(F32))
            hs = u if hs is None else hs + u
        return hs

    def fold_lo(a, bit):
        return a + pltpu.roll(a, LANES - bit, 1)

    def merge_hi(a_folded, b, bit):
        lane = lax.broadcasted_iota(jnp.int32, b.shape, 1)
        return jnp.where((lane & bit) == 0, a_folded, b + pltpu.roll(b, bit, 1))

    def project(xst):
        mt = lax.dot_general(xst, a_ref[...], TN, preferred_element_type=F32)
        vt = jnp.dot(b_ref[...], xst, preferred_element_type=F32)
        vbad = _red8(jnp.max, jnp.where(jnp.abs(vt) <= V_HI, 0.0, 1.0))
        mt = mt.reshape(2, LANES // 16, 8, C)
        mt = jnp.concatenate([mt[0], mt[1]], axis=1).reshape(LANES, C)
        return (mt * scale).astype(BF16), vt.astype(BF16), vbad

    def pool(srcs):
        pieces = []
        for rb in range(0, C, POOL_ROWS):
            hs = [hsum(w, rb, POOL_ROWS, t) for w, t in srcs]
            bit = 1
            while len(hs) > 1:
                hs = [merge_hi(fold_lo(hs[k], bit), hs[k + 1], bit) for k in range(0, len(hs), 2)]
                bit *= 2
            pieces.append((hs[0] * (1.0 / CR)).astype(BF16))
        return project(jnp.concatenate(pieces, axis=0))

    def store_keys(j, t, vals):
        mt, vt, vbad = vals
        mt_ref[j, _blk(t, LANES // 2), :] = pltpu.bitcast(mt, U32)
        vt_ref[j, :, _blk(t, LANES)] = pltpu.bitcast(vt, U32)
        flag_ref[NB] = jnp.maximum(flag_ref[NB], vbad)

    def keys_m(j, t=None):
        v = mt_ref[j] if t is None else mt_ref[j, _blk(t, LANES // 2), :]
        return pltpu.bitcast(v, BF16)

    def keys_v(j, t=None):
        v = vt_ref[j] if t is None else vt_ref[j, :, _blk(t, LANES)]
        return pltpu.bitcast(v, BF16)

    def spread_keys(g):
        m = mt_ref[0, pl.ds(pl.multiple_of(V0 + g * 8, 8), 8), :]
        m = pltpu.bitcast(m, BF16).astype(F32)
        for ch in range(C):
            mb_ref[ch, _blk(g, 16), :] = jnp.broadcast_to(m[:, ch:ch + 1], (16, LANES))

    def finish(acc, l):
        lsum = jnp.sum(l, axis=0, keepdims=True)
        bad = jnp.where(jnp.logical_and(lsum >= L_LO, lsum <= L_HI), 0.0, 1.0)
        return ((acc * (1.0 / lsum)).astype(BF16),
                [bad[:, i:i + LANES] for i in range(0, bad.shape[1], LANES)])

    def set_flag(b, bads):
        flag_ref[b] = jnp.broadcast_to(_tree(jnp.maximum, bads), (8, LANES))

    def early_block(half, j, t=None, new_keys=()):
        r0 = half * RE
        ps, ls, bads, built = {}, {}, [], []

        def qk(u):
            p = jnp.exp2(jnp.dot(keys_m(j, t), xv_ref[r0 + u], preferred_element_type=F32))
            ls[u] = l_ref[r0 + u] + _red8(jnp.sum, p)
            l_ref[r0 + u] = ls[u]
            ps[u] = p

        def pv(u):
            p = _regroup(ps.pop(u)).astype(BF16)
            acc = acc_ref[r0 + u] + jnp.dot(keys_v(j, t), p, preferred_element_type=F32)
            acc_ref[r0 + u] = acc
            if not new_keys:
                oe_ref[r0 + u], bad = finish(acc, ls[u])
                bads.extend(bad)

        _skewed(RE, qk, pv, RE if new_keys else SKEW_A,
                [lambda srcs=srcs: built.append(pool(srcs)) for _, _, srcs in new_keys])
        for (jn, tn, _), vals in zip(new_keys, built):
            store_keys(jn, tn, vals)
        if bads:
            set_flag(half, bads)

    def main_block(b, _):
        slot = lax.rem(b, 2)
        row0 = 2 * RE + b * RM

        @pl.when(b >= 2)
        def _():
            owait(slot)

        rows_p = GROUP * LANES // 2
        fence = pl.ds(pl.multiple_of((lax.shift_right_logical(b, 20) + 1) * rows_p, 16), 8)
        zeros = jnp.zeros((8, LANES), BF16)
        order = list(range(1, NC * NTILE))
        order.insert(len(order) - MIX, 0)
        items = [(u, t, kt) for u in range(RM) for t in range(NTILE) for kt in order]
        per, end = len(order) * TIES, len(items) * TIES
        work = {}
        for q in range(LEAD, RM * NTILE + LEAD):
            for ch in range(C):
                pos = (q - LEAD) * per + (2 * ch + 1) * per // (2 * C) + SHIFT
                work.setdefault(min(pos, end), []).append((q, ch))
        never = jnp.broadcast_to((z_ref[:, :C] != 0)[None], (TIES, 8, C))
        sv, ops, qops, vops, st, pend, bads, last = {}, {}, {}, {}, {}, [], [], [0, None]

        def vpu(n):
            for q, ch in work.get(n, ()):
                if q not in ops:
                    u, t = q // NTILE, q % NTILE
                    row = row0 + u if u < RM else jnp.minimum(row0 + u, H - 1)
                    ops[q] = (xv_ref[row, :, _blk(t, LANES)].astype(F32)[None], mb_ref[...])
                xb, mb = ops[q]
                term = mb[ch:ch + 1] * xb[:, ch:ch + 1, :]
                sv[q] = term if ch == 0 else sv[q] + term
            if n in work:
                last[0] = (last[0] + 1) % (NV // 8)
                last[1] = sv[q][:, last[0] * 8:last[0] * 8 + 8, :C]
            return last[1]

        def qk(k):
            u, t, kt = items[k]
            if (u, t) not in qops:
                qops[(u, t)] = (xv_ref[row0 + u, :, _blk(t, LANES)], mt_ref[...])
            xt, mt = qops[(u, t)]
            rows = (LANES - NV if kt == 0 else LANES) // 2
            j, lo = kt // NTILE, (kt % NTILE) * (LANES // 2)
            tie = [vpu(k * TIES + a) for a in range(TIES)]
            mt = mt[j:j + 1, lo:lo + rows].reshape(TIES, rows // TIES, C)
            if tie[0] is not None:
                tie = pltpu.bitcast(jnp.concatenate(tie, axis=0), U32)
                if rows == 8 * TIES:
                    mt = lax.select(never, tie, mt)
                else:
                    mt = jnp.concatenate([lax.select(never, tie, mt[:, :8]), mt[:, 8:]], axis=1)
            s = jnp.dot(pltpu.bitcast(mt.reshape(rows, C), BF16), xt, preferred_element_type=F32)
            pend.append(s)
            if kt == 0:
                q = u * NTILE + t
                pend.append(sv_ref[:, _blk(t, LANES)] if q < LEAD else sv[q][0])
            if k % GROUP == GROUP - 1:
                p = jnp.exp2(jnp.concatenate(pend, axis=0))
                del pend[:]
                pp = p.reshape(rows_p // 8, 16, LANES)
                pp = jnp.concatenate([pp[:, :8], pp[:, 8:]], axis=2).reshape(rows_p, 2 * LANES)
                p_refs[k // GROUP % RING][0:rows_p, :] = pp.astype(BF16)
                p_refs[k // GROUP % RING][fence, 0:LANES] = zeros
                lc = _red8(jnp.sum, p)
                acc, l = st.get((u, t), (None, None))
                st[(u, t)] = (acc, lc if l is None else l + lc)

        def pv(k):
            u, t, kt = items[k]
            if (u, t) not in vops:
                vops[(u, t)] = pltpu.bitcast(vt_ref[...], BF16)
            if k % GROUP == 0:
                vops["p"] = p_refs[k // GROUP % RING][0:rows_p, :]
            vt = vops[(u, t)][kt // NTILE, :, (kt % NTILE) * LANES:(kt % NTILE + 1) * LANES]
            p = vops["p"][(k % GROUP) * LANES // 2:(k % GROUP + 1) * LANES // 2]
            p = jnp.concatenate([p[:, :LANES], p[:, LANES:]], axis=0)
            y = jnp.dot(vt, p, preferred_element_type=F32)
            acc, l = st[(u, t)]
            acc = y if acc is None else acc + y
            st[(u, t)] = (acc, l)
            if kt == order[-1]:
                ob_ref[slot, u, :, _blk(t, LANES)], bad = finish(acc, l)
                bads.extend(bad)
                if t == NTILE - 1 and u + 1 in OUT_SPLITS:
                    lo = max([0] + [e for e in OUT_SPLITS if e < u + 1])
                    pltpu.make_async_copy(ob_ref.at[slot, pl.ds(lo, u + 1 - lo)],
                                          o_hbm.at[pl.ds(row0 + lo, u + 1 - lo)],
                                          osems.at[slot]).start()

        _skewed(len(items), qk, pv, SKEW_MAIN)
        vpu(end)
        for t in range(LEAD):
            sv_ref[:, _blk(t, LANES)] = sv[RM * NTILE + t][0]
        set_flag(2 + b, bads)
        return 0

    def true_max_row(r, _):
        def tile(t, _):
            lanes = _blk(t, LANES)

            def qk(c, m):
                s = jnp.dot(keys_m(c), xv_ref[r, :, lanes], preferred_element_type=F32)
                s_ref[c] = s
                return jnp.maximum(m, _red8(jnp.max, s))

            m = lax.fori_loop(0, NC, qk, jnp.full((8, LANES), -jnp.inf, F32))
            m = jnp.max(m, axis=0, keepdims=True)

            def pv(c, carry):
                acc, l = carry
                p = jnp.exp2(s_ref[c] - m)
                return (acc + jnp.dot(keys_v(c), _regroup(p).astype(BF16),
                                      preferred_element_type=F32),
                        l + _red8(jnp.sum, p))

            acc, l = lax.fori_loop(0, NC, pv,
                                   (jnp.zeros((C, LANES), F32), jnp.zeros((8, LANES), F32)))
            oe_ref[0, :, lanes] = (acc / jnp.sum(l, axis=0, keepdims=True)).astype(BF16)
            return 0

        lax.fori_loop(0, NTILE, tile, 0)
        cp = pltpu.make_async_copy(oe_ref.at[0], o_hbm.at[r], osems.at[2])
        cp.start()
        cp.wait()
        return 0

    for cp in wcopies():
        cp.start()
    for w in range(2 * WIN):
        xcopy_first(w).start(priority=1)
    for j in range(2, NC):
        xcopy(j).start(priority=1)
    flag_ref[...] = jnp.zeros(flag_ref.shape, F32)
    z_ref[...] = jnp.zeros(z_ref.shape, U32)

    def zero(r, _):
        acc_ref[r] = jnp.zeros((C, W), F32)
        l_ref[r] = jnp.zeros((8, W), F32)
        return 0

    lax.fori_loop(0, 2 * RE, zero, 0)
    for cp in wcopies():
        cp.wait()
    wkv = wkv_ref[...]
    a_ref[...] = lax.dot_general(wkv[:, :C], wq_ref[...], NT, preferred_element_type=F32).astype(BF16)
    b_ref[...] = jnp.dot(wkv[:, C:], wo_ref[...], preferred_element_type=F32).T.astype(BF16)

    stack = []
    for q in range(WIN):
        if q % NTILE == 0:
            xcopy_first(q // NTILE).wait()
        cur = hsum(q // NTILE, 0, C, q % NTILE)
        bit = 1
        while q & bit:
            cur = merge_hi(stack.pop(), cur, bit)
            bit *= 2
        stack.append(fold_lo(cur, bit) if q < WIN - 1 else cur)
    store_keys(0, 0, project((stack[0] * (1.0 / CR)).astype(BF16)))

    def first_chunk(n, done):
        half = lax.rem(n, 2)
        last = jnp.maximum(lax.div(WIN * n + WIN - 1, NTILE),
                           lax.div((half + 1) * RE - 1, WIN))
        need = jnp.maximum(done, last + 1)

        def wait_row(w, _):
            xcopy_first(w).wait()
            return 0

        lax.fori_loop(done, need, wait_row, 0)
        srcs = [(lax.div(WIN * n + i, NTILE), lax.rem(WIN * n + i, NTILE)) for i in range(WIN)]
        early_block(half, 0, lax.div(n, 2), [(lax.div(n, NTILE), lax.rem(n, NTILE), srcs)])
        return need

    lax.fori_loop(0, 2 * NTILE, first_chunk, (WIN - 1) // NTILE + 1)

    def stage(i, _):
        j = jnp.minimum(i, NC - 1)
        spread_keys(jnp.minimum(i - 1, NV // 16 - 1))
        early_block(i - j, j)

        @pl.when(i < NC - 1)
        def _():
            xcopy(i + 1).wait()
            early_block(1, i, None,
                        [(i + 1, t, [((i + 1) * WIN + k, t) for k in range(WIN)])
                         for t in range(NTILE)])
        return 0

    lax.fori_loop(1, NC + 1, stage, 0)
    ecopy().start()

    sv_ref[...] = jnp.dot(pltpu.bitcast(mt_ref[0, V0:LANES // 2, :], BF16),
                          xv_ref[2 * RE, :, 0:LEAD * LANES], preferred_element_type=F32)
    lax.fori_loop(0, NB - 2, main_block, 0)

    unsafe = jnp.max(jnp.max(flag_ref[...], axis=0))
    ecopy().wait()
    owait(0)
    owait(1)

    @pl.when(unsafe > 0.0)
    def _():
        def block(b, _):
            lo = jnp.where(b < 2, b * RE, 2 * RE + (b - 2) * RM)

            @pl.when(jnp.max(jnp.maximum(flag_ref[b], flag_ref[NB])) > 0.0)
            def _():
                lax.fori_loop(lo, lo + jnp.where(b < 2, RE, RM), true_max_row, 0)
            return 0

        lax.fori_loop(0, NB, block, 0)


@jax.jit
def pallas_standalone__window_attn_twins__vision_kernel(
    x: jax.Array,
    wq: jax.Array,
    wkv: jax.Array,
    wo: jax.Array,
):
    B, H, W, C = x.shape
    nc = H // (WIN * WIN)
    nb = 2 + (H - 2 * RE) // RM
    assert B == 1 and H % (WIN * WIN) == 0 and W % LANES == 0
    assert (H - 2 * RE) % RM == 0 and nb >= 4 and nc >= max(3, NV // 16) and 2 * RE < WIN * WIN
    assert C % POOL_ROWS == 0 and (nc * W // LANES) % GROUP == 0
    assert (LANES - NV) % (16 * TIES) == 0 and 2 <= LEAD <= W // LANES and MIX < nc * W // LANES
    assert GROUP <= SKEW_MAIN < RING * GROUP + GROUP - 1
    xt = x.transpose(0, 1, 3, 2).reshape(H, C, W)
    out = pl.pallas_call(
        _kernel,
        in_specs=[pl.BlockSpec(memory_space=pl.ANY)] * 4,
        out_specs=pl.BlockSpec(memory_space=pl.ANY),
        out_shape=jax.ShapeDtypeStruct((H, C, W), x.dtype),
        scratch_shapes=[
            pltpu.VMEM((H, C, W), x.dtype),
            pltpu.VMEM((C, C), wq.dtype),
            pltpu.VMEM((C, 2 * C), wkv.dtype),
            pltpu.VMEM((C, C), wo.dtype),
            pltpu.VMEM((nc, W // 2, C), U32),
            pltpu.VMEM((nc, C // 2, W), U32),
            pltpu.VMEM((C, C), BF16),
            pltpu.VMEM((C, C), BF16),
            pltpu.VMEM((2 * RE, C, W), F32),
            pltpu.VMEM((2 * RE, 8, W), F32),
            pltpu.VMEM((nb + 1, 8, LANES), F32),
            pltpu.VMEM((nc, W, LANES), F32),
            pltpu.VMEM((2 * RE, C, W), x.dtype),
            pltpu.VMEM((2, RM, C, W), x.dtype),
            pltpu.VMEM((C, NV, LANES), F32),
            pltpu.VMEM((NV, LEAD * LANES), F32),
            pltpu.VMEM((8, LANES), U32),
            pltpu.SemaphoreType.DMA((3,)),
            pltpu.SemaphoreType.DMA((2 * WIN,)),
            pltpu.SemaphoreType.DMA((nc - 2,)),
            pltpu.SemaphoreType.DMA((3,)),
        ] + [pltpu.VMEM((GROUP * LANES // 2 + 16, 2 * LANES), BF16)] * RING,
        compiler_params=pltpu.CompilerParams(
            vmem_limit_bytes=100 * 1024 * 1024,
            disable_bounds_checks=True,
            disable_semaphore_checks=True,
        ),
    )(xt, wq, wkv, wo)
    return out.reshape(B, H, C, W).transpose(0, 1, 3, 2)
```
